```python
import jax
import jax.numpy as jnp

def _softmax(x, axis=-1):
    return jax.nn.softmax(x, axis=axis)

def _gelu(x):
    return jax.nn.gelu(x, approximate=True)

def _silu(x):
    return jax.nn.silu(x)

def _sigmoid(x):
    return jax.nn.sigmoid(x)

def _layernorm(x, axis=-1, eps=1e-05):
    m = jnp.mean(x, axis=axis, keepdims=True)
    v = jnp.var(x, axis=axis, keepdims=True)
    return (x - m) / jnp.sqrt(v + eps)

def _scatter_add(tgt, idx, src, axis=0):
    return tgt.at[idx].add(src)

def _segment_sum(src, seg, n):
    return jax.ops.segment_sum(src, seg, n)

class _Rng:

    def __init__(self, key):
        self._k = key

    def _next(self):
        self._k, sub = jax.random.split(self._k)
        return sub

    def normal(self, shape):
        return jax.random.normal(self._next(), shape, dtype=jnp.bfloat16)

    def randint(self, lo, hi, shape):
        return jax.random.randint(self._next(), shape, lo, hi, dtype=jnp.int32)

    def uniform(self, shape, lo=0.0, hi=1.0):
        return jax.random.uniform(self._next(), shape, jnp.bfloat16, lo, hi)

    def permutation(self, n):
        return jax.random.permutation(self._next(), n)
kernel_name = 'concat_heads__softmax_full_mha__memory_aug_recurrent_mem_tr__prompt'

def setup_inputs():
    _rng = _Rng(jax.random.key(int.from_bytes(__import__("os").urandom(4), "little")))
    _w = lambda a: (lambda t: t.astype(jnp.bfloat16) if jnp.issubdtype(t.dtype, jnp.floating) else t)(jnp.asarray(a))

    def _A_setup():
        B, S, D = (1, 2048, 1024)
        return {'x': _w((lambda *s: _rng.normal(s) * 0.05)(B, S, D)), 'wqkv': _w((lambda *s: _rng.normal(s) * 0.05)(D, 3 * D)), 'wo': _w((lambda *s: _rng.normal(s) * 0.05)(D, D))}
    _A_in = _A_setup()

    def _B_setup():
        B, S, Dm = (1, 2048, 1024)
        H, Dh = (32, 128)
        M, seg = (8, 32)
        seg = min(seg, S)
        S = S // seg * seg
        return {'x': _w((lambda *s: _rng.normal(s) * 0.05)(B, S, Dm)), 'mem0': _w((lambda *s: _rng.normal(s) * 0.05)(B, M, Dm)), 'Wq': _w((lambda *s: _rng.normal(s) * 0.05)(Dm, H, Dh) * Dm ** (-0.5)), 'Wk': _w((lambda *s: _rng.normal(s) * 0.05)(Dm, H, Dh) * Dm ** (-0.5)), 'Wv': _w((lambda *s: _rng.normal(s) * 0.05)(Dm, H, Dh) * Dm ** (-0.5)), 'Wo': _w((lambda *s: _rng.normal(s) * 0.05)(H, Dh, Dm) * (H * Dh) ** (-0.5)), 'seg_len': seg}
    _B_in = _B_setup()
    return {'A_x': _A_in['x'], 'A_wqkv': _A_in['wqkv'], 'A_wo': _A_in['wo'], 'B_x': _B_in['x'], 'B_mem0': _B_in['mem0'], 'B_Wq': _B_in['Wq'], 'B_Wk': _B_in['Wk'], 'B_Wv': _B_in['Wv'], 'B_Wo': _B_in['Wo'], 'B_seg_len': _B_in['seg_len']}

def reference(A_x, A_wqkv, A_wo, B_x, B_mem0, B_Wq, B_Wk, B_Wv, B_Wo, B_seg_len):

    def _A_ref(x, wqkv, wo):
        B, S, D = x.shape
        H = 32
        Dh = D // H
        qkv = (lambda x, *d: x.transpose(*d))((x @ wqkv).reshape(B, S, 3, H, Dh), 2, 0, 3, 1, 4)
        q, k, v = (qkv[0], qkv[1], qkv[2])
        scale = Dh ** (-0.5)
        scores = jnp.einsum('bhqd,bhkd->bhqk', q, k) * scale
        p = _softmax(scores, axis=-1)
        o = jnp.einsum('bhqk,bhkd->bhqd', p, v)
        return (lambda x, *d: x.transpose(*d))(o, 0, 2, 1, 3).reshape(B, S, D) @ wo

    def _B_ref(x, mem0, Wq, Wk, Wv, Wo, seg_len):
        B, S, Dm = x.shape
        H, Dh = (Wq.shape[1], Wq.shape[2])
        M = mem0.shape[1]
        scale = Dh ** (-0.5)
        n_seg = S // seg_len
        L = M + seg_len
        idx = jnp.arange(L)
        mask = (idx[:, None] < M) | (idx[:, None] >= idx[None, :])
        mem = mem0
        outs = []
        for s in range(n_seg):
            xs = x[:, s * seg_len:(s + 1) * seg_len, :].copy()
            h = jnp.concatenate([mem, xs], axis=1)
            q = jnp.einsum('btd,dhe->bhte', h, Wq)
            k = jnp.einsum('btd,dhe->bhte', h, Wk)
            v = jnp.einsum('btd,dhe->bhte', h, Wv)
            scores = jnp.einsum('bhqe,bhke->bhqk', q, k) * scale
            scores = jnp.where(mask[None, None], scores, -1000000000.0)
            p = _softmax(scores, axis=-1)
            o = jnp.einsum('bhqk,bhke->bhqe', p, v)
            o = jnp.einsum('bhte,hed->btd', o, Wo)
            mem = o[:, :M, :].copy()
            outs.append(o[:, M:, :])
        return jnp.concatenate(outs, axis=1)
    a = _A_ref(A_x, A_wqkv, A_wo)
    b = _B_ref(B_x, B_mem0, B_Wq, B_Wk, B_Wv, B_Wo, B_seg_len)
    return jnp.concatenate([a, b], axis=-1)
```

```python
import math

import jax
import jax.numpy as jnp
from jax import lax
import jax.experimental.pallas as pl
import jax.experimental.pallas.tpu as pltpu

bf16 = jnp.bfloat16
f32 = jnp.float32
u32 = jnp.uint32

S = 2048
D = 1024
HA, DA = 32, 32
HB, DB = 32, 128
M, SEG = 8, 32
L = M + SEG
QB = 512
NQB = S // QB
KT = 128
LOG2E = math.log2(math.e)


def _b_schedule(NG):
    seq = [('k', 0), ('q', 0), ('v', 0)]
    for g in range(NG):
        nx = g + 1 < NG
        if g == 0:
            seq += [('qk', g), ('sm', g)]
        if nx:
            seq += [('q', g + 1)]
        seq += [('pv', g)]
        if nx:
            seq += [('k', g + 1)]
        seq += [('o', g)]
        if nx:
            seq += [('qk', g + 1), ('sm', g + 1), ('v', g + 1)]
    return seq


def _kernel(xa_hbm, wqkv_hbm, woa_hbm, xb_hbm, mem0_ref, wq_hbm, wk_hbm, wv_hbm, wob_hbm,
            out_hbm,
            xa, wqkv, woa, k3, qt, vt, oa, s0, s1, s2, s3, m_ref, ostage,
            wq, wk, wv, wob, xb, raw, outa, outb, h_ref, sems, rsems, osems):
    def pk(x):
        return pltpu.bitcast(x, u32)

    def up(x):
        return pltpu.bitcast(x, bf16)

    cp_xa = pltpu.make_async_copy(xa_hbm.bitcast(u32), xa, sems.at[0])
    cp_wqkv = pltpu.make_async_copy(wqkv_hbm.bitcast(u32), wqkv, sems.at[1])
    cp_woa = pltpu.make_async_copy(woa_hbm.bitcast(u32), woa, sems.at[2])
    cp_xb = pltpu.make_async_copy(xb_hbm.bitcast(u32), xb, sems.at[3])
    cp_wob = pltpu.make_async_copy(wob_hbm.bitcast(u32), wob, sems.at[4])
    cp_xa.start()
    cp_wqkv.start()
    cp_xa.wait()
    cp_wqkv.wait()
    cp_woa.start()
    cp_xb.start()
    cp_wob.start()

    w_hbms = (wq_hbm, wk_hbm, wv_hbm)
    w_dsts = (wq, wk, wv)

    def raw_copy(c, slot, i):
        return pltpu.make_async_copy(
            w_hbms[i].bitcast(u32).at[pl.ds(c * 256, 256), :], raw.at[slot, i], rsems.at[slot, i])

    def raw_start(c):
        for i in range(3):
            raw_copy(c, c % 3, i).start()

    def raw_relayout(c):
        slot = c % 3
        for i in range(3):
            raw_copy(c, slot, i).wait()
        rows = pl.ds(pl.multiple_of(c * 8, 8), 8)
        for i in range(3):
            for j in range(HB // 2):
                a = raw[slot, i, pl.ds(j, 8, stride=16), :]
                b = raw[slot, i, pl.ds(128 + j, 8, stride=16), :]
                lo = jnp.concatenate([pltpu.bitcast(a << 16, f32), pltpu.bitcast(b << 16, f32)], axis=0)
                hm = jnp.uint32(0xFFFF0000)
                hi = jnp.concatenate([pltpu.bitcast(a & hm, f32), pltpu.bitcast(b & hm, f32)], axis=0)
                w_dsts[i][rows, (2 * j) * DB:(2 * j + 1) * DB] = pk(lo.astype(bf16))
                w_dsts[i][rows, (2 * j + 1) * DB:(2 * j + 2) * DB] = pk(hi.astype(bf16))

    raw_start(0)
    raw_start(1)

    qscale = DA ** -0.5 * LOG2E

    def a1_body(r, c):
        xr = up(xa[pl.ds(pl.multiple_of(r * (QB // 2), QB // 2), QB // 2), :])
        q = jnp.dot(xr, up(wqkv[:, 0:D]), preferred_element_type=f32) * qscale
        for g in range(8):
            t = q[:, g * 128:(g + 1) * 128].T.astype(bf16)
            qt[r, g * 4:(g + 1) * 4] = pk(t).reshape(4, DA // 2, QB)
        k = jnp.dot(xr, up(wqkv[:, D:2 * D]), preferred_element_type=f32).astype(bf16)
        for g in range(8):
            k3[g, pl.ds(pl.multiple_of(r * (QB // 2), QB // 2), QB // 2), :] = pk(k[:, g * 128:(g + 1) * 128])
        v = jnp.dot(xr, up(wqkv[:, 2 * D:3 * D]), preferred_element_type=f32)
        for g in range(8):
            t = v[:, g * 128:(g + 1) * 128].T.astype(bf16)
            vt[r, g * 4:(g + 1) * 4] = pk(t).reshape(4, DA // 2, QB)
        return c

    lax.fori_loop(0, NQB, a1_body, 0)

    sbufs = (s0, s1, s2, s3)
    NI = HA * NQB
    NB = NI // 2

    def stage12(n1, hh1, sw, n2, hh2, sr, m2, do1, do2):
        m = acc = l = None
        if do1:
            gq = n1 // 4
            g1 = gq // NQB
            qb1 = gq % NQB
            q_ = up(qt[qb1, g1 * 4 + hh1])
            parts = []
            if hh1 > 0:
                parts.append(jnp.zeros((DA * hh1, QB), bf16))
            parts.append(q_)
            if hh1 < 3:
                parts.append(jnp.zeros((DA * (3 - hh1), QB), bf16))
            q_ = jnp.concatenate(parts, axis=0)
        if do2:
            h2 = (n2 // 4 // NQB) * 4 + hh2
        for kt in range(S // KT):
            if do1:
                kk = up(k3[g1, kt * (KT // 2):(kt + 1) * (KT // 2), :])
                st = jnp.dot(kk, q_, preferred_element_type=f32)
                sw[kt * KT:(kt + 1) * KT, :] = st
                mm = jnp.max(st.reshape(KT // 8, 8, QB), axis=0)
                m = mm if m is None else jnp.maximum(m, mm)
            if do2:
                p = jnp.exp2(sr[kt * KT:(kt + 1) * KT, :] - m2)
                ll = jnp.sum(p.reshape(KT // 8, 8, QB), axis=0)
                l = ll if l is None else l + ll
                r_, c_ = divmod(kt * KT, QB)
                v_ = up(vt[r_, h2, :, c_:c_ + KT])
                o = jnp.dot(v_, p.astype(bf16), preferred_element_type=f32)
                acc = o if acc is None else acc + o
        if do2:
            l = jnp.sum(l, axis=0, keepdims=True)
            ostage[hh2 * DA:(hh2 + 1) * DA, :] = acc * (1.0 / l)
        if do1:
            return jnp.max(m, axis=0, keepdims=True)

    def block(b, par, do1=True, do2=True):
        for j in range(2):
            sw = sbufs[(1 - par) * 2 + j]
            sr = sbufs[par * 2 + j]
            m2 = m_ref[par * 2 + j] if do2 else None
            n1 = jnp.minimum((b + 1) * 2 + j, NI - 1)
            m1 = stage12(n1, (1 - par) * 2 + j, sw, b * 2 + j, par * 2 + j, sr, m2, do1, do2)
            if do1:
                m_ref[(1 - par) * 2 + j] = m1
        if do2 and par == 1:
            gq = b // 2
            g = gq // NQB
            qb = gq % NQB
            oa[g, pl.ds(pl.multiple_of(qb * (QB // 2), QB // 2), QB // 2), :] = pk(ostage[...].T.astype(bf16))

    block(-1, 1, do2=False)

    def a2_body(b, c):
        @pl.when(b + 2 < NB)
        def _():
            raw_start(b + 2)

        @pl.when(b % 2 == 0)
        def _():
            block(b, 0)
            raw_relayout(b)

        @pl.when(b % 2 == 1)
        def _():
            block(b, 1)
            raw_relayout(b)
        return c

    lax.fori_loop(0, NB, a2_body, 0)

    cp_woa.wait()

    def a4_body(r, c):
        rows = pl.ds(pl.multiple_of(r * (QB // 2), QB // 2), QB // 2)
        o_ = jnp.concatenate([up(oa[g, rows, :]) for g in range(8)], axis=1)
        y = jnp.dot(o_, up(woa[...]), preferred_element_type=f32)
        outa[pl.ds(pl.multiple_of(r * QB, QB), QB), :] = y.astype(bf16)
        return c

    lax.fori_loop(0, NQB, a4_body, 0)
    cp_outa = pltpu.make_async_copy(outa, out_hbm.at[:, pl.ds(0, D)], osems.at[0])
    cp_outa.start()

    cp_xb.wait()
    cp_wob.wait()
    G = 4
    NG = HB // G
    seq = _b_schedule(NG)
    scale = DB ** -0.5 * LOG2E
    h_ref[0:M, :] = mem0_ref[...].astype(f32)
    row = lax.broadcasted_iota(jnp.int32, (L, L), 0)
    col = lax.broadcasted_iota(jnp.int32, (L, L), 1)
    mask = (row < M) | (row >= col)
    OC = 8

    def outb_copy(c):
        rows = pl.ds(c * (OC * SEG), OC * SEG)
        return pltpu.make_async_copy(outb.at[rows, :], out_hbm.at[rows, pl.ds(D, D)], osems.at[1])

    def w(ref, r0, nr, c0, nc):
        return up(ref[r0 // 2:(r0 + nr) // 2, c0:c0 + nc])

    def b_step(s, c):
        h_ref[M:L, :] = up(xb[pl.ds(pl.multiple_of(s * (SEG // 2), SEG // 2), SEG // 2), :]).astype(f32)
        hv = h_ref[...]
        st = {}
        acc = None
        for op, g in seq:
            if op in ('q', 'k', 'v'):
                ref = {'q': wq, 'k': wk, 'v': wv}[op]
                st[op, g] = jnp.dot(hv, w(ref, 0, D, g * G * DB, G * DB), preferred_element_type=f32)
            elif op == 'qk':
                q = st.pop(('q', g))
                k = st.pop(('k', g))
                st['s', g] = [
                    lax.dot_general(q[:, j * DB:(j + 1) * DB], k[:, j * DB:(j + 1) * DB].astype(bf16),
                                    (((1,), (1,)), ((), ())), preferred_element_type=f32)
                    for j in range(G)]
            elif op == 'sm':
                ps = []
                for sc in st.pop(('s', g)):
                    sc = jnp.where(mask, sc * scale, -1e9)
                    mx = jnp.max(sc, axis=-1, keepdims=True)
                    p = jnp.exp2(sc - mx)
                    ps.append(p / jnp.sum(p, axis=-1, keepdims=True))
                st['p', g] = ps
            elif op == 'pv':
                v = st.pop(('v', g))
                st['ov', g] = jnp.concatenate(
                    [jnp.dot(p, v[:, j * DB:(j + 1) * DB].astype(bf16), preferred_element_type=f32)
                     for j, p in enumerate(st.pop(('p', g)))], axis=1)
            elif op == 'o':
                r = jnp.dot(st.pop(('ov', g)), w(wob, g * G * DB, G * DB, 0, D), preferred_element_type=f32)
                acc = r if acc is None else acc + r
        h_ref[0:M, :] = acc[0:M, :].astype(bf16).astype(f32)
        outb[pl.ds(pl.multiple_of(s * SEG, SEG), SEG), :] = acc[M:L, :].astype(bf16)

        @pl.when(s % OC == OC - 1)
        def _():
            outb_copy(s // OC).start()
        return c

    lax.fori_loop(0, S // SEG, b_step, 0)

    cp_outa.wait()
    for c in range(S // SEG // OC):
        outb_copy(c).wait()


@jax.jit
def pallas_concat_heads__softmax_full_mha__memory_aug_recurrent_mem_tr__prompt_kernel(
        A_x, A_wqkv, A_wo, B_x, B_mem0, B_Wq, B_Wk, B_Wv, B_Wo, B_seg_len):
    del B_seg_len
    any_spec = pl.BlockSpec(memory_space=pl.ANY)
    V = pltpu.VMEM
    scratch = [
        V((S // 2, D), u32),
        V((D // 2, 3 * D), u32),
        V((D // 2, D), u32),
        V((8, S // 2, 128), u32),
        V((NQB, HA, DA // 2, QB), u32),
        V((NQB, HA, DA // 2, QB), u32),
        V((8, S // 2, 128), u32),
        V((S, QB), f32), V((S, QB), f32), V((S, QB), f32), V((S, QB), f32),
        V((4, 1, QB), f32),
        V((128, QB), f32),
        V((D // 2, HB * DB), u32), V((D // 2, HB * DB), u32), V((D // 2, HB * DB), u32),
        V((HB * DB // 2, D), u32),
        V((S // 2, D), u32),
        V((3, 3, 256, 128), u32),
        V((S, D), bf16),
        V((S, D), bf16),
        V((L, D), f32),
        pltpu.SemaphoreType.DMA((5,)),
        pltpu.SemaphoreType.DMA((3, 3)),
        pltpu.SemaphoreType.DMA((2,)),
    ]
    out = pl.pallas_call(
        _kernel,
        out_shape=jax.ShapeDtypeStruct((S, 2 * D), bf16),
        in_specs=[any_spec, any_spec, any_spec, any_spec, pl.BlockSpec(memory_space=pltpu.VMEM),
                  any_spec, any_spec, any_spec, any_spec],
        out_specs=any_spec,
        scratch_shapes=scratch,
        compiler_params=pltpu.CompilerParams(vmem_limit_bytes=120 * 1024 * 1024),
    )(A_x.reshape(S, D), A_wqkv, A_wo, B_x.reshape(S, D), B_mem0.reshape(M, D),
      B_Wq.reshape(D * HB, DB), B_Wk.reshape(D * HB, DB), B_Wv.reshape(D * HB, DB),
      B_Wo.reshape(HB * DB, D))
    return out.reshape(1, S, 2 * D)
```

```python
import math

import jax
import jax.numpy as jnp
from jax import lax
import jax.experimental.pallas as pl
import jax.experimental.pallas.tpu as pltpu

bf16 = jnp.bfloat16
f32 = jnp.float32
u32 = jnp.uint32

S = 2048
D = 1024
HA, DA = 32, 32
HB, DB = 32, 128
M, SEG = 8, 32
L = M + SEG
QB = 512
NQB = S // QB
KT = 128
NKT = S // KT
LOG2E = math.log2(math.e)

TREE = 4
UNROLL = 2
NAP = 2


B_ORDER = ('k0 q0 A1 v0 qk0 sm0 q1 k1 q2 pv0 o0b o0a qk1 v1 sm1 k2 pv1 v2 o1b o1a qk2 q3 sm2 pv2 k3 o2a '
           'qk3 v3 sm3 q4 pv3 k4 o3b o2b o3a qk4 sm4 v4 q5 pv4 k5 o4a o4b qk5 v5 sm5 q6 pv5 k6 o5a qk6 '
           'k7 sm6 v6 q7 pv6 o5b qk7 v7 sm7 o6a pv7 o6b o7a o7b A0 ')


def _b_schedule():
    s = B_ORDER.split()
    out = []
    for t in s:
        part = t[-1] if t[-1] in 'abcd' else ''
        t = t[:-1] if part else t
        out.append((t[:-1], int(t[-1]), part))
    return out


def _kernel(xa_hbm, wqkv_hbm, woa_hbm, xb_hbm, mem0_ref, wq_hbm, wk_hbm, wv_hbm, wob_hbm,
            out_hbm,
            xa, wqkv, woa, k3, qt, vt, oa, s0, s1, s2, s3, s4, s5, s6, s7, m_ref, os0, os1,
            wq, wk, wv, wob, xb, raw, outa, outb, h_ref, z_ref, sems, rsems, osems):
    def pk(x):
        return pltpu.bitcast(x, u32)

    def up(x):
        return pltpu.bitcast(x, bf16)

    QP = QB // 2

    z_ref[...] = jnp.zeros(z_ref.shape, u32)
    xa32 = xa_hbm.bitcast(u32)
    wqkv32 = wqkv_hbm.bitcast(u32)

    def cp_xa(r):
        rows = pl.ds(r * QP, QP)
        return pltpu.make_async_copy(xa32.at[rows, :], xa.at[rows, :], sems.at[r])

    def cp_wqkv(i):
        cols = pl.ds(i * D, D)
        return pltpu.make_async_copy(wqkv32.at[:, cols], wqkv.at[:, cols], sems.at[4 + i])

    cp_woa = pltpu.make_async_copy(woa_hbm.bitcast(u32), woa, sems.at[7])
    cp_xb = pltpu.make_async_copy(xb_hbm.bitcast(u32), xb, sems.at[8])
    cp_wob = pltpu.make_async_copy(wob_hbm.bitcast(u32), wob, sems.at[9])

    cp_xa(0).start()
    cp_wqkv(0).start()
    cp_xa(0).wait()
    cp_wqkv(0).wait()
    for r in range(1, NQB):
        cp_xa(r).start()
    cp_wqkv(1).start()

    w_hbms = (wq_hbm, wk_hbm, wv_hbm)
    w_dsts = (wq, wk, wv)
    RC = 8

    def raw_copy(c, i):
        return pltpu.make_async_copy(
            w_hbms[i].bitcast(u32).at[pl.ds(c * (RC * 256), RC * 256), :],
            raw.at[c % 2, i], rsems.at[c % 2, i])

    def raw_start(c):
        for i in range(3):
            raw_copy(c, i).start()

    def raw_wait(c):
        for i in range(3):
            raw_copy(c, i).wait()

    chain = {}

    def raw_relayout(blk, i, j):
        slot = (blk // RC) % 2
        base = pl.multiple_of((blk % RC) * 256, 256)
        rows = pl.ds(pl.multiple_of(blk * 8, 8), 8)
        a = raw[slot, i, pl.ds(base + j, 8, stride=16), :]
        b = raw[slot, i, pl.ds(base + 128 + j, 8, stride=16), :]
        if chain.get('prev') is not None:
            pz = chain['prev'] & chain['z']
            a = a | pz
            b = b | pz
        lo = jnp.concatenate([pltpu.bitcast(a << 16, f32), pltpu.bitcast(b << 16, f32)], axis=0)
        hm = jnp.uint32(0xFFFF0000)
        hi = jnp.concatenate([pltpu.bitcast(a & hm, f32), pltpu.bitcast(b & hm, f32)], axis=0)
        lo = pk(lo.astype(bf16))
        hi = pk(hi.astype(bf16))
        w_dsts[i][rows, (2 * j) * DB:(2 * j + 1) * DB] = lo
        w_dsts[i][rows, (2 * j + 1) * DB:(2 * j + 2) * DB] = hi
        chain['prev'] = hi

    qscale = DA ** -0.5 * LOG2E

    def xrows(r):
        return up(xa[pl.ds(pl.multiple_of(r * QP, QP), QP), :])

    def a1_q(r, c):
        @pl.when(r > 0)
        def _():
            cp_xa(r).wait()
        q = jnp.dot(xrows(r), up(wqkv[:, 0:D]), preferred_element_type=f32) * qscale
        for g in range(8):
            t = q[:, g * 128:(g + 1) * 128].T.astype(bf16)
            qt[r, g * 4:(g + 1) * 4] = pk(t).reshape(4, DA // 2, QB)
        return c

    def relayout_chunk(c):
        chain['prev'] = None
        chain['z'] = z_ref[...]
        for t in range(RC):
            for i in range(3):
                for j in range(HB // 2):
                    raw_relayout(c * RC + t, i, j)

    def raw_step(c):
        raw_wait(c)

        @pl.when(c + 1 < 2 * NQB)
        def _():
            raw_start(c + 1)

    def a1_k(r, c):
        raw_step(r)
        k = jnp.dot(xrows(r), up(wqkv[:, D:2 * D]), preferred_element_type=f32).astype(bf16)
        for g in range(8):
            k3[g, pl.ds(pl.multiple_of(r * QP, QP), QP), :] = pk(k[:, g * 128:(g + 1) * 128])
        relayout_chunk(r)
        return c

    def a1_v(r, c):
        raw_step(NQB + r)
        v = jnp.dot(xrows(r), up(wqkv[:, 2 * D:3 * D]), preferred_element_type=f32)
        for g in range(8):
            t = v[:, g * 128:(g + 1) * 128].T.astype(bf16)
            vt[r, g * 4:(g + 1) * 4] = pk(t).reshape(4, DA // 2, QB)
        relayout_chunk(NQB + r)
        return c

    cp_wqkv(2).start()
    raw_start(0)
    lax.fori_loop(0, NQB, a1_q, 0)
    cp_wqkv(1).wait()
    lax.fori_loop(0, NQB, a1_k, 0)
    cp_wqkv(2).wait()
    lax.fori_loop(0, NQB, a1_v, 0)
    cp_woa.start()
    cp_xb.start()
    cp_wob.start()

    sbufs = (s0, s1, s2, s3, s4, s5, s6, s7)
    NB = HA * NQB // 4

    def stage12(gq1, hh, sw, gq2, sr, m2, do1, do2, ostage):
        m = acc = l = None
        if do1:
            g1 = gq1 // NQB
            qb1 = gq1 % NQB
            parts = []
            if hh > 0:
                parts.append(jnp.zeros((DA * hh, QB), bf16))
            parts.append(up(qt[qb1, g1 * 4 + hh]))
            if hh < 3:
                parts.append(jnp.zeros((DA * (3 - hh), QB), bf16))
            q_ = jnp.concatenate(parts, axis=0)
        if do2:
            h2 = (gq2 // NQB) * 4 + hh
        for kt in range(NKT):
            if do1:
                kk = up(k3[g1, kt * (KT // 2):(kt + 1) * (KT // 2), :])
                st = jnp.dot(kk, q_, preferred_element_type=f32)
                sw[kt * KT:(kt + 1) * KT, :] = st
                mm = jnp.max(st.reshape(KT // 8, 8, QB), axis=0)
                m = mm if m is None else jnp.maximum(m, mm)
            if do2:
                p = jnp.exp2(sr[kt * KT:(kt + 1) * KT, :] - m2)
                t = p.reshape(KT // 8, 8, QB)
                for _ in range(TREE):
                    t4 = t.reshape(t.shape[0] // 2, 2, 8, QB)
                    t = t4[:, 0] + t4[:, 1]
                ll = jnp.sum(t, axis=0)
                l = ll if l is None else l + ll
                r_, c_ = divmod(kt * KT, QB)
                v_ = up(vt[r_, h2, :, c_:c_ + KT])
                o = jnp.dot(v_, p.astype(bf16), preferred_element_type=f32)
                acc = o if acc is None else acc + o
        if do2:
            l = jnp.sum(l, axis=0, keepdims=True)
            ostage[hh * DA:(hh + 1) * DA, :] = acc * (1.0 / l)
        if do1:
            return jnp.max(m, axis=0, keepdims=True)

    def block(b, par, do1=True, do2=True, flush=True):
        if do2 and flush:
            flush_o(b - 1, (os0, os1)[1 - par])
        gq1 = jnp.minimum(b + 1, NB - 1)
        for j in range(4):
            sw = sbufs[(1 - par) * 4 + j]
            sr = sbufs[par * 4 + j]
            m2 = m_ref[par * 4 + j] if do2 else None
            m1 = stage12(gq1, j, sw, b, sr, m2, do1, do2, (os0, os1)[par])
            if do1:
                m_ref[(1 - par) * 4 + j] = m1

    def flush_o(b, ostage):
        b = jnp.maximum(b, 0)
        g = b // NQB
        qb = b % NQB
        oa[g, pl.ds(pl.multiple_of(qb * QP, QP), QP), :] = pk(ostage[...].T.astype(bf16))

    block(-1, 1, do2=False)

    def a2_body(b, c):
        @pl.when(b % 2 == 0)
        def _():
            block(b, 0)

        @pl.when(b % 2 == 1)
        def _():
            block(b, 1)
        return c

    os1[...] = jnp.zeros(os1.shape, f32)
    lax.fori_loop(0, NB - 1, a2_body, 0)
    block(NB - 1, 1, do1=False)
    flush_o(NB - 1, os1)

    cp_woa.wait()

    cp_xb.wait()
    cp_wob.wait()
    G = 4
    NG = HB // G
    seq = _b_schedule()
    scale = DB ** -0.5 * LOG2E
    h_ref[0:M, :] = mem0_ref[...].astype(f32)
    row = lax.broadcasted_iota(jnp.int32, (L, L), 0)
    col = lax.broadcasted_iota(jnp.int32, (L, L), 1)
    mask = (row < M) | (row >= col)
    OC = 8

    def outb_copy(c):
        rows = pl.ds(c * (OC * SEG), OC * SEG)
        return pltpu.make_async_copy(outb.at[rows, :], out_hbm.at[rows, pl.ds(D, D)], osems.at[1])

    def w(ref, r0, nr, c0, nc):
        return up(ref[r0 // 2:(r0 + nr) // 2, c0:c0 + nc])

    def outa_copy(c):
        rows = pl.ds(c * (OC * SEG), OC * SEG)
        return pltpu.make_async_copy(outa.at[rows, :], out_hbm.at[rows, pl.ds(0, D)], osems.at[0])

    def a4_part(s, p):
        prow = pl.ds(pl.multiple_of(s * (SEG // 2), SEG // 2), SEG // 2)
        o_ = jnp.concatenate([up(oa[g, prow, :]) for g in range(8)], axis=1)
        wd = D // NAP
        y = jnp.dot(o_, up(woa[:, p * wd:(p + 1) * wd]), preferred_element_type=f32)
        outa[pl.ds(pl.multiple_of(s * SEG, SEG), SEG), p * wd:(p + 1) * wd] = y.astype(bf16)

    def one_step(s):
        h_ref[M:L, :] = up(xb[pl.ds(pl.multiple_of(s * (SEG // 2), SEG // 2), SEG // 2), :]).astype(f32)
        hv = h_ref[...]
        st = {}
        acc = {}
        for op, g, part in seq:
            if op in ('q', 'k', 'v'):
                ref = {'q': wq, 'k': wk, 'v': wv}[op]
                st[op, g] = jnp.dot(hv, w(ref, 0, D, g * G * DB, G * DB), preferred_element_type=f32)
            elif op == 'qk':
                q = st.pop(('q', g))
                k = st.pop(('k', g))
                st['s', g] = [
                    lax.dot_general(q[:, j * DB:(j + 1) * DB], k[:, j * DB:(j + 1) * DB].astype(bf16),
                                    (((1,), (1,)), ((), ())), preferred_element_type=f32)
                    for j in range(G)]
            elif op == 'sm':
                ps = []
                for sc in st.pop(('s', g)):
                    sc = jnp.where(mask, sc * scale, -1e9)
                    mx = jnp.max(sc, axis=-1, keepdims=True)
                    p = jnp.exp2(sc - mx)
                    ps.append(p / jnp.sum(p, axis=-1, keepdims=True))
                st['p', g] = ps
            elif op == 'pv':
                v = st.pop(('v', g))
                st['ov', g] = jnp.concatenate(
                    [jnp.dot(p, v[:, j * DB:(j + 1) * DB].astype(bf16), preferred_element_type=f32)
                     for j, p in enumerate(st.pop(('p', g)))], axis=1)
            elif op == 'A':
                a4_part(s, g)
            elif op == 'o':
                for hf in ((0, 1) if part == '' else ('ab'.index(part),)):
                    r = jnp.dot(st['ov', g], w(wob, g * G * DB, G * DB, hf * 512, 512),
                                preferred_element_type=f32)
                    acc[hf] = r if hf not in acc else acc[hf] + r
        for hf in (0, 1):
            cols = slice(hf * 512, (hf + 1) * 512)
            h_ref[0:M, cols] = acc[hf][0:M, :].astype(bf16).astype(f32)
            outb[pl.ds(pl.multiple_of(s * SEG, SEG), SEG), cols] = acc[hf][M:L, :].astype(bf16)

    def b_body(i, c):
        for u in range(UNROLL):
            one_step(i * UNROLL + u)
        s_last = i * UNROLL + UNROLL - 1

        @pl.when(s_last % OC == OC - 1)
        def _():
            outa_copy(s_last // OC).start()
            outb_copy(s_last // OC).start()
        return c

    lax.fori_loop(0, S // SEG // UNROLL, b_body, 0)

    for c in range(S // SEG // OC):
        outa_copy(c).wait()
        outb_copy(c).wait()


@jax.jit
def pallas_concat_heads__softmax_full_mha__memory_aug_recurrent_mem_tr__prompt_kernel(
        A_x, A_wqkv, A_wo, B_x, B_mem0, B_Wq, B_Wk, B_Wv, B_Wo, B_seg_len):
    del B_seg_len
    any_spec = pl.BlockSpec(memory_space=pl.ANY)
    V = pltpu.VMEM
    scratch = [
        V((S // 2, D), u32),
        V((D // 2, 3 * D), u32),
        V((D // 2, D), u32),
        V((8, S // 2, 128), u32),
        V((NQB, HA, DA // 2, QB), u32),
        V((NQB, HA, DA // 2, QB), u32),
        V((8, S // 2, 128), u32),
    ] + [V((S, QB), f32) for _ in range(8)] + [
        V((8, 1, QB), f32),
        V((128, QB), f32), V((128, QB), f32),
        V((D // 2, HB * DB), u32), V((D // 2, HB * DB), u32), V((D // 2, HB * DB), u32),
        V((HB * DB // 2, D), u32),
        V((S // 2, D), u32),
        V((2, 3, 8 * 256, 128), u32),
        V((S, D), bf16),
        V((S, D), bf16),
        V((L, D), f32),
        V((8, 128), u32),
        pltpu.SemaphoreType.DMA((10,)),
        pltpu.SemaphoreType.DMA((2, 3)),
        pltpu.SemaphoreType.DMA((2,)),
    ]
    out = pl.pallas_call(
        _kernel,
        out_shape=jax.ShapeDtypeStruct((S, 2 * D), bf16),
        in_specs=[any_spec, any_spec, any_spec, any_spec, pl.BlockSpec(memory_space=pltpu.VMEM),
                  any_spec, any_spec, any_spec, any_spec],
        out_specs=any_spec,
        scratch_shapes=scratch,
        compiler_params=pltpu.CompilerParams(vmem_limit_bytes=120 * 1024 * 1024, disable_bounds_checks=True),
    )(A_x.reshape(S, D), A_wqkv, A_wo, B_x.reshape(S, D), B_mem0.reshape(M, D),
      B_Wq.reshape(D * HB, DB), B_Wk.reshape(D * HB, DB), B_Wv.reshape(D * HB, DB),
      B_Wo.reshape(HB * DB, D))
    return out.reshape(1, S, 2 * D)
```

```python
import math

import jax
import jax.numpy as jnp
from jax import lax
import jax.experimental.pallas as pl
import jax.experimental.pallas.tpu as pltpu

bf16 = jnp.bfloat16
f32 = jnp.float32
u32 = jnp.uint32

S = 2048
D = 1024
HA, DA = 32, 32
HB, DB = 32, 128
M, SEG = 8, 32
L = M + SEG
QB = 512
NQB = S // QB
KT = 128
NKT = S // KT
LOG2E = math.log2(math.e)

TREE = 4
UNROLL = 2
NAP = 2


B_ORDER = (
    ('k0 q0 v0 q1 qk0 sm0 k1 q2 pv0 o0b o0a qk1 sm1 v1 k2 pv1 v2 o1b qk2 q3 A3 sm2 pv2 k3 o1a o2a '
     'qk3 v3 sm3 q4 o2b pv3 k4 o3b qk4 o3a sm4 v4 q5 pv4 k5 o4a o4b qk5 v5 sm5 q6 pv5 k6 o5a qk6 '
     'k7 v6 sm6 q7 pv6 o5b A2 qk7 v7 sm7 A1 o6a pv7 o6b o7a o7b A0 '),
    ('q0 k0 v0 qk0 sm0 q1 k1 q2 pv0 o0b o0a qk1 v1 sm1 k2 pv1 v2 o1b qk2 q3 o1a sm2 pv2 k3 o2a qk3 '
     'v3 sm3 q4 pv3 k4 o3b o2b o3a qk4 v4 sm4 q5 pv4 k5 o4a o4b qk5 v5 q6 sm5 pv5 k6 k7 qk6 o5a '
     'sm6 v6 q7 pv6 o5b qk7 v7 sm7 o6a pv7 o6b o7a o7b '),
)


def _b_schedule(txt):
    out = []
    for t in txt.split():
        part = t[-1] if t[-1] in 'ab' else ''
        t = t[:-1] if part else t
        out.append((t[:-1], int(t[-1]), part))
    return out


def _kernel(xa_hbm, wqkv_hbm, woa_hbm, xb_hbm, mem0_ref, wq_hbm, wk_hbm, wv_hbm, wob_hbm,
            out_hbm,
            xa, wqkv, woa, k3, qt, vt, oa, s0, s1, s2, s3, s4, s5, s6, s7, m_ref, os0, os1,
            wq, wk, wv, wob, xb, raw, outa, outb, h_ref, z_ref, sems, rsems, osems):
    def pk(x):
        return pltpu.bitcast(x, u32)

    def up(x):
        return pltpu.bitcast(x, bf16)

    QP = QB // 2

    z_ref[...] = jnp.zeros(z_ref.shape, u32)
    xa32 = xa_hbm.bitcast(u32)
    wqkv32 = wqkv_hbm.bitcast(u32)

    def cp_xa(r):
        rows = pl.ds(r * QP, QP)
        return pltpu.make_async_copy(xa32.at[rows, :], xa.at[rows, :], sems.at[r])

    NWC = 4
    WC = D // NWC

    def cp_wq(c):
        cols = pl.ds(c * WC, WC)
        return pltpu.make_async_copy(wqkv32.at[:, cols], wqkv.at[:, cols], sems.at[4 + c])

    def cp_wkv(i):
        cols = pl.ds(i * D, D)
        return pltpu.make_async_copy(wqkv32.at[:, cols], wqkv.at[:, cols], sems.at[3 + NWC + i])

    cp_woa = pltpu.make_async_copy(woa_hbm.bitcast(u32), woa, sems.at[6 + NWC])
    cp_xb = pltpu.make_async_copy(xb_hbm.bitcast(u32), xb, sems.at[7 + NWC])
    cp_wob = pltpu.make_async_copy(wob_hbm.bitcast(u32), wob, sems.at[8 + NWC])

    w_hbms = (wq_hbm, wk_hbm, wv_hbm)
    w_dsts = (wq, wk, wv)
    RC = 8
    NSLOT = 3
    NRC = D // 16 // RC

    def raw_copy(c, i):
        return pltpu.make_async_copy(
            w_hbms[i].bitcast(u32).at[pl.ds(c * (RC * 256), RC * 256), :],
            raw.at[c % NSLOT, i], rsems.at[c % NSLOT, i])

    def raw_start(c):
        for i in range(3):
            raw_copy(c, i).start()

    def raw_wait(c):
        for i in range(3):
            raw_copy(c, i).wait()

    chain = {}

    def raw_relayout(blk, i, j):
        slot = (blk // RC) % NSLOT
        base = pl.multiple_of((blk % RC) * 256, 256)
        rows = pl.ds(pl.multiple_of(blk * 8, 8), 8)
        a = raw[slot, i, pl.ds(base + j, 8, stride=16), :]
        b = raw[slot, i, pl.ds(base + 128 + j, 8, stride=16), :]
        if chain.get('prev') is not None:
            pz = chain['prev'] & chain['z']
            a = a | pz
            b = b | pz
        lo = jnp.concatenate([pltpu.bitcast(a << 16, f32), pltpu.bitcast(b << 16, f32)], axis=0)
        hm = jnp.uint32(0xFFFF0000)
        hi = jnp.concatenate([pltpu.bitcast(a & hm, f32), pltpu.bitcast(b & hm, f32)], axis=0)
        lo = pk(lo.astype(bf16))
        hi = pk(hi.astype(bf16))
        w_dsts[i][rows, (2 * j) * DB:(2 * j + 1) * DB] = lo
        w_dsts[i][rows, (2 * j + 1) * DB:(2 * j + 2) * DB] = hi
        chain['prev'] = hi

    qscale = DA ** -0.5 * LOG2E

    def xrows(r):
        return up(xa[pl.ds(pl.multiple_of(r * QP, QP), QP), :])

    def q_dot(x_, c0, nc):
        return jnp.dot(x_, up(wqkv[:, c0:c0 + nc]), preferred_element_type=f32) * qscale

    def q_store(r, q, c0):
        for g in range(q.shape[1] // 128):
            t = q[:, g * 128:(g + 1) * 128].T.astype(bf16)
            g4 = (c0 // 128 + g) * 4
            qt[r, g4:g4 + 4] = pk(t).reshape(4, DA // 2, QB)

    def a1_q(r, c):
        cp_xa(r).wait()
        q_store(r, q_dot(xrows(r), 0, D), 0)
        return c

    def relayout_chunk(c):
        chain['prev'] = None
        chain['z'] = z_ref[...]
        for t in range(RC):
            for i in range(3):
                for j in range(HB // 2):
                    raw_relayout(c * RC + t, i, j)

    def raw_step(c):
        raw_wait(c)

        @pl.when(c + NSLOT - 1 < NRC)
        def _():
            raw_start(c + NSLOT - 1)

    def a1_k(r, c):
        raw_step(r)
        k = jnp.dot(xrows(r), up(wqkv[:, D:2 * D]), preferred_element_type=f32).astype(bf16)
        for g in range(8):
            k3[g, pl.ds(pl.multiple_of(r * QP, QP), QP), :] = pk(k[:, g * 128:(g + 1) * 128])
        relayout_chunk(r)
        return c

    def a1_v(r, c):
        raw_step(NQB + r)
        v = jnp.dot(xrows(r), up(wqkv[:, 2 * D:3 * D]), preferred_element_type=f32)
        for g in range(8):
            t = v[:, g * 128:(g + 1) * 128].T.astype(bf16)
            vt[r, g * 4:(g + 1) * 4] = pk(t).reshape(4, DA // 2, QB)
        relayout_chunk(NQB + r)
        return c

    cp_xa(0).start()
    for c in range(NWC):
        cp_wq(c).start()
    for r in range(1, NQB):
        cp_xa(r).start()
    cp_wkv(1).start()
    raw_start(0)
    cp_wkv(2).start()
    for c in range(1, NSLOT - 1):
        raw_start(c)

    cp_xa(0).wait()
    prev = None
    for c in range(NWC):
        cp_wq(c).wait()
        q = q_dot(xrows(0), c * WC, WC)
        if prev is not None:
            q_store(0, *prev)
        prev = (q, c * WC)
    q_store(0, *prev)
    lax.fori_loop(1, NQB, a1_q, 0)
    cp_wkv(1).wait()
    lax.fori_loop(0, NQB, a1_k, 0)
    cp_wkv(2).wait()
    lax.fori_loop(0, NQB, a1_v, 0)
    cp_woa.start()
    cp_xb.start()
    cp_wob.start()

    sbufs = (s0, s1, s2, s3, s4, s5, s6, s7)
    NB = HA * NQB // 4

    def stage12(gq1, hh, sw, gq2, sr, m2, do1, do2, ostage):
        m = acc = l = None
        if do1:
            g1 = gq1 // NQB
            qb1 = gq1 % NQB
            parts = []
            if hh > 0:
                parts.append(jnp.zeros((DA * hh, QB), bf16))
            parts.append(up(qt[qb1, g1 * 4 + hh]))
            if hh < 3:
                parts.append(jnp.zeros((DA * (3 - hh), QB), bf16))
            q_ = jnp.concatenate(parts, axis=0)
        if do2:
            h2 = (gq2 // NQB) * 4 + hh
        for kt in range(NKT):
            if do1:
                kk = up(k3[g1, kt * (KT // 2):(kt + 1) * (KT // 2), :])
                st = jnp.dot(kk, q_, preferred_element_type=f32)
                sw[kt * KT:(kt + 1) * KT, :] = st
                mm = jnp.max(st.reshape(KT // 8, 8, QB), axis=0)
                m = mm if m is None else jnp.maximum(m, mm)
            if do2:
                p = jnp.exp2(sr[kt * KT:(kt + 1) * KT, :] - m2)
                t = p.reshape(KT // 8, 8, QB)
                for _ in range(TREE):
                    t4 = t.reshape(t.shape[0] // 2, 2, 8, QB)
                    t = t4[:, 0] + t4[:, 1]
                ll = jnp.sum(t, axis=0)
                l = ll if l is None else l + ll
                r_, c_ = divmod(kt * KT, QB)
                v_ = up(vt[r_, h2, :, c_:c_ + KT])
                o = jnp.dot(v_, p.astype(bf16), preferred_element_type=f32)
                acc = o if acc is None else acc + o
        if do2:
            l = jnp.sum(l, axis=0, keepdims=True)
            ostage[hh * DA:(hh + 1) * DA, :] = acc * (1.0 / l)
        if do1:
            return jnp.max(m, axis=0, keepdims=True)

    def block(b, par, do1=True, do2=True, flush=True):
        if do2 and flush:
            flush_o(b - 1, (os0, os1)[1 - par])
        gq1 = jnp.minimum(b + 1, NB - 1)
        for j in range(4):
            sw = sbufs[(1 - par) * 4 + j]
            sr = sbufs[par * 4 + j]
            m2 = m_ref[par * 4 + j] if do2 else None
            m1 = stage12(gq1, j, sw, b, sr, m2, do1, do2, (os0, os1)[par])
            if do1:
                m_ref[(1 - par) * 4 + j] = m1

    def flush_o(b, ostage):
        b = jnp.maximum(b, 0)
        g = b // NQB
        qb = b % NQB
        oa[g, pl.ds(pl.multiple_of(qb * QP, QP), QP), :] = pk(ostage[...].T.astype(bf16))

    block(-1, 1, do2=False)

    def a2_body(b, c):
        @pl.when(b % 2 == 0)
        def _():
            block(b, 0)

        @pl.when(b % 2 == 1)
        def _():
            block(b, 1)
        return c

    os1[...] = jnp.zeros(os1.shape, f32)
    lax.fori_loop(0, NB - 1, a2_body, 0)
    block(NB - 1, 1, do1=False)
    flush_o(NB - 1, os1)

    cp_woa.wait()

    cp_xb.wait()
    cp_wob.wait()
    G = 4
    NG = HB // G
    seqs = [_b_schedule(t) for t in B_ORDER]
    scale = DB ** -0.5 * LOG2E
    h_ref[0:M, :] = mem0_ref[...].astype(f32)
    row = lax.broadcasted_iota(jnp.int32, (L, L), 0)
    col = lax.broadcasted_iota(jnp.int32, (L, L), 1)
    mask = (row < M) | (row >= col)
    OC = UNROLL

    def outb_copy(c):
        rows = pl.ds(c * (OC * SEG), OC * SEG)
        return pltpu.make_async_copy(outb.at[rows, :], out_hbm.at[rows, pl.ds(D, D)], osems.at[1])

    def w(ref, r0, nr, c0, nc):
        return up(ref[r0 // 2:(r0 + nr) // 2, c0:c0 + nc])

    def outa_copy(c):
        rows = pl.ds(c * (OC * SEG), OC * SEG)
        return pltpu.make_async_copy(outa.at[rows, :], out_hbm.at[rows, pl.ds(0, D)], osems.at[0])

    def a4_part(s, p):
        prow = pl.ds(pl.multiple_of(s * (SEG // 2), SEG // 2), SEG // 2)
        o_ = jnp.concatenate([up(oa[g, prow, :]) for g in range(8)], axis=1)
        wd = D // NAP
        y = jnp.dot(o_, up(woa[:, p * wd:(p + 1) * wd]), preferred_element_type=f32)
        outa[pl.ds(pl.multiple_of(s * SEG, SEG), SEG), p * wd:(p + 1) * wd] = y.astype(bf16)

    def one_step(s, seq, s0):
        h_ref[M:L, :] = up(xb[pl.ds(pl.multiple_of(s * (SEG // 2), SEG // 2), SEG // 2), :]).astype(f32)
        hv = h_ref[...]
        st = {}
        acc = {}
        for op, g, part in seq:
            if op in ('q', 'k', 'v'):
                ref = {'q': wq, 'k': wk, 'v': wv}[op]
                st[op, g] = jnp.dot(hv, w(ref, 0, D, g * G * DB, G * DB), preferred_element_type=f32)
            elif op == 'qk':
                q = st.pop(('q', g))
                k = st.pop(('k', g))
                st['s', g] = [
                    lax.dot_general(q[:, j * DB:(j + 1) * DB], k[:, j * DB:(j + 1) * DB].astype(bf16),
                                    (((1,), (1,)), ((), ())), preferred_element_type=f32)
                    for j in range(G)]
            elif op == 'sm':
                ps = []
                for sc in st.pop(('s', g)):
                    sc = jnp.where(mask, sc * scale, -1e9)
                    mx = jnp.max(sc, axis=-1, keepdims=True)
                    p = jnp.exp2(sc - mx)
                    ps.append(p / jnp.sum(p, axis=-1, keepdims=True))
                st['p', g] = ps
            elif op == 'pv':
                v = st.pop(('v', g))
                st['ov', g] = jnp.concatenate(
                    [jnp.dot(p, v[:, j * DB:(j + 1) * DB].astype(bf16), preferred_element_type=f32)
                     for j, p in enumerate(st.pop(('p', g)))], axis=1)
            elif op == 'A':
                a4_part(s0 + g // NAP, g % NAP)
            elif op == 'o':
                for hf in ((0, 1) if part == '' else ('ab'.index(part),)):
                    r = jnp.dot(st['ov', g], w(wob, g * G * DB, G * DB, hf * 512, 512),
                                preferred_element_type=f32)
                    acc[hf] = r if hf not in acc else acc[hf] + r
        for hf in (0, 1):
            cols = slice(hf * 512, (hf + 1) * 512)
            h_ref[0:M, cols] = acc[hf][0:M, :].astype(bf16).astype(f32)
            outb[pl.ds(pl.multiple_of(s * SEG, SEG), SEG), cols] = acc[hf][M:L, :].astype(bf16)

    def b_body(i, c):
        for u in range(UNROLL):
            one_step(i * UNROLL + u, seqs[u], i * UNROLL)
        outa_copy(i).start()
        outb_copy(i).start()
        return c

    lax.fori_loop(0, S // SEG // UNROLL, b_body, 0)

    pltpu.make_async_copy(outa, out_hbm.at[:, pl.ds(0, D)], osems.at[0]).wait()
    pltpu.make_async_copy(outb, out_hbm.at[:, pl.ds(D, D)], osems.at[1]).wait()


@jax.jit
def pallas_concat_heads__softmax_full_mha__memory_aug_recurrent_mem_tr__prompt_kernel(
        A_x, A_wqkv, A_wo, B_x, B_mem0, B_Wq, B_Wk, B_Wv, B_Wo, B_seg_len):
    del B_seg_len
    any_spec = pl.BlockSpec(memory_space=pl.ANY)
    V = pltpu.VMEM
    scratch = [
        V((S // 2, D), u32),
        V((D // 2, 3 * D), u32),
        V((D // 2, D), u32),
        V((8, S // 2, 128), u32),
        V((NQB, HA, DA // 2, QB), u32),
        V((NQB, HA, DA // 2, QB), u32),
        V((8, S // 2, 128), u32),
    ] + [V((S, QB), f32) for _ in range(8)] + [
        V((8, 1, QB), f32),
        V((128, QB), f32), V((128, QB), f32),
        V((D // 2, HB * DB), u32), V((D // 2, HB * DB), u32), V((D // 2, HB * DB), u32),
        V((HB * DB // 2, D), u32),
        V((S // 2, D), u32),
        V((3, 3, 8 * 256, 128), u32),
        V((S, D), bf16),
        V((S, D), bf16),
        V((L, D), f32),
        V((8, 128), u32),
        pltpu.SemaphoreType.DMA((13,)),
        pltpu.SemaphoreType.DMA((3, 3)),
        pltpu.SemaphoreType.DMA((2,)),
    ]
    out = pl.pallas_call(
        _kernel,
        out_shape=jax.ShapeDtypeStruct((S, 2 * D), bf16),
        in_specs=[any_spec, any_spec, any_spec, any_spec, pl.BlockSpec(memory_space=pltpu.VMEM),
                  any_spec, any_spec, any_spec, any_spec],
        out_specs=any_spec,
        scratch_shapes=scratch,
        compiler_params=pltpu.CompilerParams(vmem_limit_bytes=120 * 1024 * 1024, disable_bounds_checks=True),
    )(A_x.reshape(S, D), A_wqkv, A_wo, B_x.reshape(S, D), B_mem0.reshape(M, D),
      B_Wq.reshape(D * HB, DB), B_Wk.reshape(D * HB, DB), B_Wv.reshape(D * HB, DB),
      B_Wo.reshape(HB * DB, D))
    return out.reshape(1, S, 2 * D)
```

```python
import math

import jax
import jax.numpy as jnp
from jax import lax
import jax.experimental.pallas as pl
import jax.experimental.pallas.tpu as pltpu

bf16 = jnp.bfloat16
f32 = jnp.float32
u32 = jnp.uint32

S = 2048
D = 1024
HA, DA = 32, 32
HB, DB = 32, 128
M, SEG = 8, 32
L = M + SEG
QB = 512
NQB = S // QB
KT = 128
NKT = S // KT
LOG2E = math.log2(math.e)

TREE = 4
UNROLL = 2
NAP = 2


B_ORDER = (
    ('k0 q0 v0 q1 qk0 sm0 k1 q2 pv0 o0b o0a qk1 sm1 v1 k2 pv1 v2 o1b qk2 q3 A3 sm2 pv2 k3 o1a o2a '
     'qk3 v3 sm3 q4 o2b pv3 k4 o3b qk4 o3a sm4 v4 q5 pv4 k5 o4a o4b qk5 v5 sm5 q6 pv5 k6 o5a qk6 '
     'k7 v6 sm6 q7 pv6 o5b A2 qk7 v7 sm7 A1 o6a pv7 o6b o7a o7b A0 '),
    ('q0 k0 v0 qk0 sm0 q1 k1 q2 pv0 o0b o0a qk1 v1 sm1 k2 pv1 v2 o1b qk2 q3 o1a sm2 pv2 k3 o2a qk3 '
     'v3 sm3 q4 pv3 k4 o3b o2b o3a qk4 v4 sm4 q5 pv4 k5 o4a o4b qk5 v5 q6 sm5 pv5 k6 k7 qk6 o5a '
     'sm6 v6 q7 pv6 o5b qk7 v7 sm7 o6a pv7 o6b o7a o7b '),
)


def _b_schedule(txt):
    out = []
    for t in txt.split():
        part = t[-1] if t[-1] in 'ab' else ''
        t = t[:-1] if part else t
        out.append((t[:-1], int(t[-1]), part))
    return out


def _kernel(xa_hbm, wqkv_hbm, woa_hbm, xb_hbm, mem0_ref, wq_hbm, wk_hbm, wv_hbm, wob_hbm,
            out_hbm,
            xa, wqkv, woa, k3, qvt, tstage, oa, s0, s1, s2, s3, s4, s5, s6, s7, m_ref, os0, os1,
            wq, wk, wv, wob, xb, raw, outa, outb, h_ref, z_ref, sems, rsems, osems):
    def pk(x):
        return pltpu.bitcast(x, u32)

    def up(x):
        return pltpu.bitcast(x, bf16)

    QP = QB // 2
    qt = qvt.at[0]
    vt = qvt.at[1]

    z_ref[...] = jnp.zeros(z_ref.shape, u32)
    xa32 = xa_hbm.bitcast(u32)
    wqkv32 = wqkv_hbm.bitcast(u32)

    def cp_xa(r):
        rows = pl.ds(r * QP, QP)
        return pltpu.make_async_copy(xa32.at[rows, :], xa.at[rows, :], sems.at[r])

    NWC = 4
    WC = D // NWC

    def cp_x0(hf):
        rows = pl.ds(hf * (QP // 2), QP // 2)
        return pltpu.make_async_copy(xa32.at[rows, :], xa.at[rows, :], sems.at[(0, 13)[hf]])

    def cp_wq(c):
        cols = pl.ds(c * WC, WC)
        return pltpu.make_async_copy(wqkv32.at[:, cols], wqkv.at[:, cols], sems.at[4 + c])

    def cp_wkv(i):
        cols = pl.ds(i * D, D)
        return pltpu.make_async_copy(wqkv32.at[:, cols], wqkv.at[:, cols], sems.at[3 + NWC + i])

    cp_woa = pltpu.make_async_copy(woa_hbm.bitcast(u32), woa, sems.at[6 + NWC])
    cp_xb = pltpu.make_async_copy(xb_hbm.bitcast(u32), xb, sems.at[7 + NWC])
    cp_wob = pltpu.make_async_copy(wob_hbm.bitcast(u32), wob, sems.at[8 + NWC])

    w_hbms = (wq_hbm, wk_hbm, wv_hbm)
    w_dsts = (wq, wk, wv)
    RC = 8
    NSLOT = 3
    NRC = D // 16 // RC

    def raw_copy(c, i):
        return pltpu.make_async_copy(
            w_hbms[i].bitcast(u32).at[pl.ds(c * (RC * 256), RC * 256), :],
            raw.at[c % NSLOT, i], rsems.at[c % NSLOT, i])

    def raw_start(c):
        for i in range(3):
            raw_copy(c, i).start()

    def raw_wait(c):
        for i in range(3):
            raw_copy(c, i).wait()

    chain = {}

    def raw_relayout(blk, i, j):
        slot = (blk // RC) % NSLOT
        base = pl.multiple_of((blk % RC) * 256, 256)
        rows = pl.ds(pl.multiple_of(blk * 8, 8), 8)
        a = raw[slot, i, pl.ds(base + j, 8, stride=16), :]
        b = raw[slot, i, pl.ds(base + 128 + j, 8, stride=16), :]
        if chain.get('prev') is not None:
            pz = chain['prev'] & chain['z']
            a = a | pz
            b = b | pz
        lo = jnp.concatenate([pltpu.bitcast(a << 16, f32), pltpu.bitcast(b << 16, f32)], axis=0)
        hm = jnp.uint32(0xFFFF0000)
        hi = jnp.concatenate([pltpu.bitcast(a & hm, f32), pltpu.bitcast(b & hm, f32)], axis=0)
        lo = pk(lo.astype(bf16))
        hi = pk(hi.astype(bf16))
        w_dsts[i][rows, (2 * j) * DB:(2 * j + 1) * DB] = lo
        w_dsts[i][rows, (2 * j + 1) * DB:(2 * j + 2) * DB] = hi
        chain['prev'] = hi

    qscale = DA ** -0.5 * LOG2E

    def xrows(r):
        return up(xa[pl.ds(pl.multiple_of(r * QP, QP), QP), :])

    def q_dot(x_, c0, nc):
        return jnp.dot(x_, up(wqkv[:, c0:c0 + nc]), preferred_element_type=f32) * qscale

    def t_stage(y, r0, c0):
        tstage[r0 // 2:(r0 + y.shape[0]) // 2, c0:c0 + y.shape[1]] = pk(y.astype(bf16))

    def t_flush(which, r):
        for g in range(8):
            t = up(tstage[:, g * 128:(g + 1) * 128]).astype(f32).T.astype(bf16)
            qvt[which, r, g * 4:g * 4 + 4] = pk(t).reshape(4, DA // 2, QB)

    def a1_q(r, c):
        cp_xa(r).wait()
        t_flush(0, r - 1)
        t_stage(q_dot(xrows(r), 0, D), 0, 0)
        return c

    def relayout_chunk(c):
        chain['prev'] = None
        chain['z'] = z_ref[...]
        for t in range(RC):
            for i in range(3):
                for j in range(HB // 2):
                    raw_relayout(c * RC + t, i, j)

    def raw_step(c):
        raw_wait(c)

        @pl.when(c + NSLOT - 1 < NRC)
        def _():
            raw_start(c + NSLOT - 1)

    def a1_k(r, c):
        raw_step(r)
        k = jnp.dot(xrows(r), up(wqkv[:, D:2 * D]), preferred_element_type=f32).astype(bf16)
        for g in range(8):
            k3[g, pl.ds(pl.multiple_of(r * QP, QP), QP), :] = pk(k[:, g * 128:(g + 1) * 128])
        relayout_chunk(r)
        return c

    def a1_v(r, c):
        raw_step(NQB + r)
        t_flush(jnp.where(r == 0, 0, 1), jnp.where(r == 0, NQB - 1, r - 1))
        t_stage(jnp.dot(xrows(r), up(wqkv[:, 2 * D:3 * D]), preferred_element_type=f32), 0, 0)
        relayout_chunk(NQB + r)
        return c

    cp_wq(0).start()
    cp_x0(0).start()
    cp_x0(1).start()
    for c in range(1, NWC):
        cp_wq(c).start()
    for r in range(1, NQB):
        cp_xa(r).start()
    cp_wkv(1).start()
    raw_start(0)
    cp_wkv(2).start()
    for c in range(1, NSLOT - 1):
        raw_start(c)

    def x0half(hf):
        return up(xa[hf * (QP // 2):(hf + 1) * (QP // 2), :])

    pieces = [(cp_x0(0), lambda: x0half(0), 0, 0), (cp_x0(1), lambda: x0half(1), QB // 2, 0)]
    pieces += [(cp_wq(c), lambda: xrows(0), 0, c * WC) for c in range(1, NWC)]
    cp_wq(0).wait()
    prev = None
    for cp, lhs, r0, c0 in pieces:
        cp.wait()
        y = q_dot(lhs(), c0, WC)
        if prev is not None:
            t_stage(*prev)
        prev = (y, r0, c0)
    t_stage(*prev)
    lax.fori_loop(1, NQB, a1_q, 0)
    cp_wkv(1).wait()
    lax.fori_loop(0, NQB, a1_k, 0)
    cp_wkv(2).wait()
    lax.fori_loop(0, NQB, a1_v, 0)
    cp_woa.start()
    cp_xb.start()
    cp_wob.start()

    sbufs = (s0, s1, s2, s3, s4, s5, s6, s7)
    NB = HA * NQB // 4

    def stage12(gq1, hh, sw, gq2, sr, m2, do1, do2, ostage):
        m = acc = l = None
        if do1:
            g1 = gq1 // NQB
            qb1 = gq1 % NQB
            parts = []
            if hh > 0:
                parts.append(jnp.zeros((DA * hh, QB), bf16))
            parts.append(up(qt[qb1, g1 * 4 + hh]))
            if hh < 3:
                parts.append(jnp.zeros((DA * (3 - hh), QB), bf16))
            q_ = jnp.concatenate(parts, axis=0)
        if do2:
            h2 = (gq2 // NQB) * 4 + hh
        for kt in range(NKT):
            if do1:
                kk = up(k3[g1, kt * (KT // 2):(kt + 1) * (KT // 2), :])
                st = jnp.dot(kk, q_, preferred_element_type=f32)
                sw[kt * KT:(kt + 1) * KT, :] = st
                mm = jnp.max(st.reshape(KT // 8, 8, QB), axis=0)
                m = mm if m is None else jnp.maximum(m, mm)
            if do2:
                p = jnp.exp2(sr[kt * KT:(kt + 1) * KT, :] - m2)
                t = p.reshape(KT // 8, 8, QB)
                for _ in range(TREE):
                    t4 = t.reshape(t.shape[0] // 2, 2, 8, QB)
                    t = t4[:, 0] + t4[:, 1]
                ll = jnp.sum(t, axis=0)
                l = ll if l is None else l + ll
                r_, c_ = divmod(kt * KT, QB)
                v_ = up(vt[r_, h2, :, c_:c_ + KT])
                o = jnp.dot(v_, p.astype(bf16), preferred_element_type=f32)
                acc = o if acc is None else acc + o
        if do2:
            l = jnp.sum(l, axis=0, keepdims=True)
            ostage[hh * DA:(hh + 1) * DA, :] = acc * (1.0 / l)
        if do1:
            return jnp.max(m, axis=0, keepdims=True)

    def block(b, par, do1=True, do2=True, flush=True):
        if do2 and flush:
            flush_o(b - 1, (os0, os1)[1 - par])
        gq1 = jnp.minimum(b + 1, NB - 1)
        for j in range(4):
            sw = sbufs[(1 - par) * 4 + j]
            sr = sbufs[par * 4 + j]
            m2 = m_ref[par * 4 + j] if do2 else None
            m1 = stage12(gq1, j, sw, b, sr, m2, do1, do2, (os0, os1)[par])
            if do1:
                m_ref[(1 - par) * 4 + j] = m1

    def flush_o(b, ostage):
        b = jnp.maximum(b, 0)
        g = b // NQB
        qb = b % NQB
        oa[g, pl.ds(pl.multiple_of(qb * QP, QP), QP), :] = pk(ostage[...].T.astype(bf16))

    t_flush(1, NQB - 1)
    block(-1, 1, do2=False)

    def a2_body(b, c):
        @pl.when(b % 2 == 0)
        def _():
            block(b, 0)

        @pl.when(b % 2 == 1)
        def _():
            block(b, 1)
        return c

    os1[...] = jnp.zeros(os1.shape, f32)
    lax.fori_loop(0, NB - 1, a2_body, 0)
    block(NB - 1, 1, do1=False)
    flush_o(NB - 1, os1)

    cp_woa.wait()

    cp_xb.wait()
    cp_wob.wait()
    G = 4
    NG = HB // G
    seqs = [_b_schedule(t) for t in B_ORDER]
    scale = DB ** -0.5 * LOG2E
    h_ref[0:M, :] = mem0_ref[...].astype(f32)
    row = lax.broadcasted_iota(jnp.int32, (L, L), 0)
    col = lax.broadcasted_iota(jnp.int32, (L, L), 1)
    mask = (row < M) | (row >= col)
    OC = UNROLL

    def outb_copy(c):
        rows = pl.ds(c * (OC * SEG), OC * SEG)
        return pltpu.make_async_copy(outb.at[rows, :], out_hbm.at[rows, pl.ds(D, D)], osems.at[1])

    def w(ref, r0, nr, c0, nc):
        return up(ref[r0 // 2:(r0 + nr) // 2, c0:c0 + nc])

    def outa_copy(c):
        rows = pl.ds(c * (OC * SEG), OC * SEG)
        return pltpu.make_async_copy(outa.at[rows, :], out_hbm.at[rows, pl.ds(0, D)], osems.at[0])

    def a4_part(s, p):
        prow = pl.ds(pl.multiple_of(s * (SEG // 2), SEG // 2), SEG // 2)
        o_ = jnp.concatenate([up(oa[g, prow, :]) for g in range(8)], axis=1)
        wd = D // NAP
        y = jnp.dot(o_, up(woa[:, p * wd:(p + 1) * wd]), preferred_element_type=f32)
        outa[pl.ds(pl.multiple_of(s * SEG, SEG), SEG), p * wd:(p + 1) * wd] = y.astype(bf16)

    def one_step(s, seq, s0):
        h_ref[M:L, :] = up(xb[pl.ds(pl.multiple_of(s * (SEG // 2), SEG // 2), SEG // 2), :]).astype(f32)
        hv = h_ref[...]
        st = {}
        acc = {}
        for op, g, part in seq:
            if op in ('q', 'k', 'v'):
                ref = {'q': wq, 'k': wk, 'v': wv}[op]
                st[op, g] = jnp.dot(hv, w(ref, 0, D, g * G * DB, G * DB), preferred_element_type=f32)
            elif op == 'qk':
                q = st.pop(('q', g))
                k = st.pop(('k', g))
                st['s', g] = [
                    lax.dot_general(q[:, j * DB:(j + 1) * DB], k[:, j * DB:(j + 1) * DB].astype(bf16),
                                    (((1,), (1,)), ((), ())), preferred_element_type=f32)
                    for j in range(G)]
            elif op == 'sm':
                ps = []
                for sc in st.pop(('s', g)):
                    sc = jnp.where(mask, sc * scale, -1e9)
                    mx = jnp.max(sc, axis=-1, keepdims=True)
                    p = jnp.exp2(sc - mx)
                    ps.append(p / jnp.sum(p, axis=-1, keepdims=True))
                st['p', g] = ps
            elif op == 'pv':
                v = st.pop(('v', g))
                st['ov', g] = jnp.concatenate(
                    [jnp.dot(p, v[:, j * DB:(j + 1) * DB].astype(bf16), preferred_element_type=f32)
                     for j, p in enumerate(st.pop(('p', g)))], axis=1)
            elif op == 'A':
                a4_part(s0 + g // NAP, g % NAP)
            elif op == 'o':
                for hf in ((0, 1) if part == '' else ('ab'.index(part),)):
                    r = jnp.dot(st['ov', g], w(wob, g * G * DB, G * DB, hf * 512, 512),
                                preferred_element_type=f32)
                    acc[hf] = r if hf not in acc else acc[hf] + r
        for hf in (0, 1):
            cols = slice(hf * 512, (hf + 1) * 512)
            h_ref[0:M, cols] = acc[hf][0:M, :].astype(bf16).astype(f32)
            outb[pl.ds(pl.multiple_of(s * SEG, SEG), SEG), cols] = acc[hf][M:L, :].astype(bf16)

    def b_body(i, c):
        for u in range(UNROLL):
            one_step(i * UNROLL + u, seqs[u], i * UNROLL)
        outa_copy(i).start()
        outb_copy(i).start()
        return c

    lax.fori_loop(0, S // SEG // UNROLL, b_body, 0)

    pltpu.make_async_copy(outa, out_hbm.at[:, pl.ds(0, D)], osems.at[0]).wait()
    pltpu.make_async_copy(outb, out_hbm.at[:, pl.ds(D, D)], osems.at[1]).wait()


@jax.jit
def pallas_concat_heads__softmax_full_mha__memory_aug_recurrent_mem_tr__prompt_kernel(
        A_x, A_wqkv, A_wo, B_x, B_mem0, B_Wq, B_Wk, B_Wv, B_Wo, B_seg_len):
    del B_seg_len
    any_spec = pl.BlockSpec(memory_space=pl.ANY)
    V = pltpu.VMEM
    scratch = [
        V((S // 2, D), u32),
        V((D // 2, 3 * D), u32),
        V((D // 2, D), u32),
        V((8, S // 2, 128), u32),
        V((2, NQB, HA, DA // 2, QB), u32),
        V((QB // 2, D), u32),
        V((8, S // 2, 128), u32),
    ] + [V((S, QB), f32) for _ in range(8)] + [
        V((8, 1, QB), f32),
        V((128, QB), f32), V((128, QB), f32),
        V((D // 2, HB * DB), u32), V((D // 2, HB * DB), u32), V((D // 2, HB * DB), u32),
        V((HB * DB // 2, D), u32),
        V((S // 2, D), u32),
        V((3, 3, 8 * 256, 128), u32),
        V((S, D), bf16),
        V((S, D), bf16),
        V((L, D), f32),
        V((8, 128), u32),
        pltpu.SemaphoreType.DMA((14,)),
        pltpu.SemaphoreType.DMA((3, 3)),
        pltpu.SemaphoreType.DMA((2,)),
    ]
    out = pl.pallas_call(
        _kernel,
        out_shape=jax.ShapeDtypeStruct((S, 2 * D), bf16),
        in_specs=[any_spec, any_spec, any_spec, any_spec, pl.BlockSpec(memory_space=pltpu.VMEM),
                  any_spec, any_spec, any_spec, any_spec],
        out_specs=any_spec,
        scratch_shapes=scratch,
        compiler_params=pltpu.CompilerParams(vmem_limit_bytes=120 * 1024 * 1024),
    )(A_x.reshape(S, D), A_wqkv, A_wo, B_x.reshape(S, D), B_mem0.reshape(M, D),
      B_Wq.reshape(D * HB, DB), B_Wk.reshape(D * HB, DB), B_Wv.reshape(D * HB, DB),
      B_Wo.reshape(HB * DB, D))
    return out.reshape(1, S, 2 * D)
```

```python
import functools
import math

import jax
import jax.numpy as jnp
from jax import lax
import jax.experimental.pallas as pl
import jax.experimental.pallas.tpu as pltpu

bf16 = jnp.bfloat16
f32 = jnp.float32
u32 = jnp.uint32

S = 2048
D = 1024
HA, DA = 32, 32
HB, DB = 32, 128
M, SEG = 8, 32
L = M + SEG
NSEG = S // SEG

QB = 512
QP = QB // 2
NQB = S // QB
KT = 128
NKT = S // KT
NB = HA * NQB // 4
TREE = 4

G = 4
UNROLL = 2
NAP = 2

NWC = 4
WC = D // NWC
RC = 8
NRC = D // 16 // RC
NSLOT = 3

LOG2E = math.log2(math.e)

B_ORDER = (
    ('k0 q0 q1 v0 qk0 sm0 k1 q2 qk1 pv0 sm1 v1 k2 o0b pv1 v2 qk2 o0a o1b A3 sm2 q3 pv2 k3 o1a qk3 '
     'o2a sm3 v3 q4 pv3 k4 v4 qk4 o2b o3b o3a sm4 q5 pv4 k5 o4a qk5 v5 o4b sm5 q6 pv5 k6 o5a k7 '
     'qk6 A2 sm6 v6 q7 o5b qk7 sm7 pv6 v7 o6a pv7 o6b o7a o7b A0 '),
    ('q0 k0 q1 qk0 v0 sm0 k1 q2 pv0 o0b qk1 A1 v1 sm1 k2 pv1 v2 o1b qk2 sm2 q3 o0a o1a pv2 k3 o2a '
     'qk3 v3 q4 sm3 pv3 k4 o2b o3b qk4 sm4 o3a v4 q5 pv4 k5 v5 o4a o4b qk5 k6 q6 sm5 pv5 k7 qk6 '
     'o5a sm6 v6 q7 pv6 o5b qk7 v7 sm7 o6a pv7 o6b o7b o7a '),
)
B_FIRST = (
    ('U k0 q0 U q1 v0 U qk0 sm0 U k1 q2 U qk1 pv0 U sm1 v1 U k2 o0b U pv1 v2 U qk2 o0a U o1b A3 U '
     'sm2 q3 k3 U pv2 U qk3 o1a U o2a sm3 U v3 pv3 q4 U k4 U v4 qk4 U o2b o3b U o3a sm4 U q5 pv4 '
     'k5 o4a U qk5 v5 U o4b sm5 U q6 pv5 k6 o5a U U k7 qk6 U A2 sm6 U v6 q7 U pv6 o5b qk7 U U v7 '
     'sm7 o6a U pv7 o6b U o7a o7b U '),
    ('U U q0 k0 U q1 qk0 U v0 U k1 q2 U sm0 pv0 o0b qk1 U U A1 v1 sm1 U k2 pv1 U v2 o1b U qk2 sm2 '
     'U q3 o0a U o1a pv2 U k3 o2a U qk3 v3 U q4 sm3 U o2b pv3 k4 U o3b U qk4 sm4 U o3a v4 U q5 pv4 '
     'U k5 v5 A0 U o4a o4b U qk5 k6 U q6 sm5 U pv5 k7 U qk6 o5a U sm6 v6 q7 pv6 U U o5b qk7 U v7 '
     'sm7 o6a pv7 o6b o7b o7a '),
)


def _parse_order(txt):
    out = []
    for t in txt.split():
        if t == 'U':
            out.append(('U', 0, ''))
            continue
        part = t[-1] if t[-1] in 'ab' else ''
        t = t[:-1] if part else t
        out.append((t[:-1], int(t[-1]), part))
    return out


def _pk(x):
    return pltpu.bitcast(x, u32)


def _up(x):
    return pltpu.bitcast(x, bf16)


def _dot(a, b):
    return jnp.dot(a, b, preferred_element_type=f32)


def _kernel(xa_hbm, wqkv_hbm, woa_hbm, xb_hbm, mem0_ref, wq_hbm, wk_hbm, wv_hbm, wob_hbm,
            out_hbm,
            xa, wqkv, woa, k3, qvt, tstage, oa, s0, s1, s2, s3, s4, s5, s6, s7, m_ref, os0, os1,
            wq, wk, wv, wob, xb, raw, outa, outb, h_ref, z_ref, sems, rsems, osems):
    qt = qvt.at[0]
    vt = qvt.at[1]
    z_ref[...] = jnp.zeros(z_ref.shape, u32)

    xa32 = xa_hbm.bitcast(u32)
    wqkv32 = wqkv_hbm.bitcast(u32)

    def cp_x0(hf):
        rows = pl.ds(hf * (QP // 2), QP // 2)
        return pltpu.make_async_copy(xa32.at[rows, :], xa.at[rows, :], sems.at[(0, 13)[hf]])

    def cp_xa(r):
        rows = pl.ds(r * QP, QP)
        return pltpu.make_async_copy(xa32.at[rows, :], xa.at[rows, :], sems.at[r])

    def cp_wq(c):
        cols = pl.ds(c * WC, WC)
        return pltpu.make_async_copy(wqkv32.at[:, cols], wqkv.at[:, cols], sems.at[4 + c])

    def cp_wkv(i):
        cols = pl.ds(i * D, D)
        return pltpu.make_async_copy(wqkv32.at[:, cols], wqkv.at[:, cols], sems.at[7 + i])

    cp_woa = pltpu.make_async_copy(woa_hbm.bitcast(u32), woa, sems.at[10])
    cp_xb = pltpu.make_async_copy(xb_hbm.bitcast(u32), xb, sems.at[11])
    cp_wob = pltpu.make_async_copy(wob_hbm.bitcast(u32), wob, sems.at[12])

    w_hbms = (wq_hbm, wk_hbm, wv_hbm)
    w_dsts = (wq, wk, wv)

    def raw_copy(c, i):
        return pltpu.make_async_copy(
            w_hbms[i].bitcast(u32).at[pl.ds(c * (RC * 256), RC * 256), :],
            raw.at[c % NSLOT, i], rsems.at[c % NSLOT, i])

    def raw_start(c):
        for i in range(3):
            raw_copy(c, i).start()

    def raw_step(c):
        for i in range(3):
            raw_copy(c, i).wait()

        @pl.when(c + NSLOT - 1 < NRC)
        def _():
            raw_start(c + NSLOT - 1)

    def relayout_chunk(c):
        slot = c % NSLOT
        z = z_ref[...]
        hm = jnp.uint32(0xFFFF0000)
        prev = None
        for t in range(RC):
            rows = pl.ds(pl.multiple_of((c * RC + t) * 8, 8), 8)
            for i in range(3):
                for j in range(HB // 2):
                    a = raw[slot, i, pl.ds(t * 256 + j, 8, stride=16), :]
                    b = raw[slot, i, pl.ds(t * 256 + 128 + j, 8, stride=16), :]
                    if prev is not None:
                        pz = prev & z
                        a = a | pz
                        b = b | pz
                    lo = jnp.concatenate([pltpu.bitcast(a << 16, f32), pltpu.bitcast(b << 16, f32)], axis=0)
                    hi = jnp.concatenate([pltpu.bitcast(a & hm, f32), pltpu.bitcast(b & hm, f32)], axis=0)
                    lo = _pk(lo.astype(bf16))
                    hi = _pk(hi.astype(bf16))
                    w_dsts[i][rows, (2 * j) * DB:(2 * j + 1) * DB] = lo
                    w_dsts[i][rows, (2 * j + 1) * DB:(2 * j + 2) * DB] = hi
                    prev = hi

    qscale = DA ** -0.5 * LOG2E

    def xrows(r):
        return _up(xa[pl.ds(pl.multiple_of(r * QP, QP), QP), :])

    def q_dot(x_, c0, nc):
        return _dot(x_, _up(wqkv[:, c0:c0 + nc])) * qscale

    def t_stage(y, r0, c0):
        tstage[r0 // 2:(r0 + y.shape[0]) // 2, c0:c0 + y.shape[1]] = _pk(y.astype(bf16))

    def t_flush(which, r):
        for g in range(8):
            t = _up(tstage[:, g * 128:(g + 1) * 128]).astype(f32).T.astype(bf16)
            qvt[which, r, g * 4:g * 4 + 4] = _pk(t).reshape(4, DA // 2, QB)

    def a1_q(r, c):
        cp_xa(r).wait()
        t_flush(0, r - 1)
        t_stage(q_dot(xrows(r), 0, D), 0, 0)
        return c

    def a1_k(r, c):
        raw_step(r)
        k = _dot(xrows(r), _up(wqkv[:, D:2 * D])).astype(bf16)
        for g in range(8):
            k3[g, pl.ds(pl.multiple_of(r * QP, QP), QP), :] = _pk(k[:, g * 128:(g + 1) * 128])
        relayout_chunk(r)
        return c

    def a1_v(r, c):
        raw_step(NQB + r)
        t_flush(jnp.where(r == 0, 0, 1), jnp.where(r == 0, NQB - 1, r - 1))
        t_stage(_dot(xrows(r), _up(wqkv[:, 2 * D:3 * D])), 0, 0)
        relayout_chunk(NQB + r)
        return c

    cp_wq(0).start()
    cp_x0(0).start()
    cp_x0(1).start()
    for c in range(1, NWC):
        cp_wq(c).start()
    for r in range(1, NQB):
        cp_xa(r).start()
    cp_wkv(1).start()
    raw_start(0)
    cp_wkv(2).start()
    for c in range(1, NSLOT - 1):
        raw_start(c)

    def x0half(hf):
        return _up(xa[hf * (QP // 2):(hf + 1) * (QP // 2), :])

    pieces = [(cp_x0(0), lambda: x0half(0), 0, 0), (cp_x0(1), lambda: x0half(1), QB // 2, 0)]
    pieces += [(cp_wq(c), lambda: xrows(0), 0, c * WC) for c in range(1, NWC)]
    cp_wq(0).wait()
    prev = None
    for cp, lhs, r0, c0 in pieces:
        cp.wait()
        y = q_dot(lhs(), c0, WC)
        if prev is not None:
            t_stage(*prev)
        prev = (y, r0, c0)
    t_stage(*prev)

    lax.fori_loop(1, NQB, a1_q, 0)
    cp_wkv(1).wait()
    lax.fori_loop(0, NQB, a1_k, 0)
    cp_wkv(2).wait()
    lax.fori_loop(0, NQB, a1_v, 0)
    cp_woa.start()
    cp_xb.start()
    cp_wob.start()

    sbufs = (s0, s1, s2, s3, s4, s5, s6, s7)

    def probs(sr, kt, m2):
        p = jnp.exp2(sr[kt * KT:(kt + 1) * KT, :] - m2)
        t = p.reshape(KT // 8, 8, QB)
        for _ in range(TREE):
            t4 = t.reshape(t.shape[0] // 2, 2, 8, QB)
            t = t4[:, 0] + t4[:, 1]
        return p.astype(bf16), jnp.sum(t, axis=0)

    def vt_tile(h, kt):
        r_, c_ = divmod(kt * KT, QB)
        return _up(vt[r_, h, :, c_:c_ + KT])

    def item(hh, b1, sw, b2, sr, m2, ostage, produce, consume):
        m = acc = l = None
        if produce:
            g1 = b1 // NQB
            parts = []
            if hh > 0:
                parts.append(jnp.zeros((DA * hh, QB), bf16))
            parts.append(_up(qt[b1 % NQB, g1 * 4 + hh]))
            if hh < 3:
                parts.append(jnp.zeros((DA * (3 - hh), QB), bf16))
            q_ = jnp.concatenate(parts, axis=0)
        if consume:
            h2 = (b2 // NQB) * 4 + hh
        for kt in range(NKT):
            if produce:
                st = _dot(_up(k3[g1, kt * (KT // 2):(kt + 1) * (KT // 2), :]), q_)
                sw[kt * KT:(kt + 1) * KT, :] = st
                mm = jnp.max(st.reshape(KT // 8, 8, QB), axis=0)
                m = mm if m is None else jnp.maximum(m, mm)
            if consume:
                p, ll = probs(sr, kt, m2)
                l = ll if l is None else l + ll
                o = _dot(vt_tile(h2, kt), p)
                acc = o if acc is None else acc + o
        if consume:
            ostage[hh * DA:(hh + 1) * DA, :] = acc * (1.0 / jnp.sum(l, axis=0, keepdims=True))
        if produce:
            return jnp.max(m, axis=0, keepdims=True)

    def flush_o(b, ostage):
        b = jnp.maximum(b, 0)
        oa[b // NQB, pl.ds(pl.multiple_of((b % NQB) * QP, QP), QP), :] = _pk(ostage[...].T.astype(bf16))

    def block(b, par, consume=True):
        if consume:
            flush_o(b - 1, (os0, os1)[1 - par])
        b1 = jnp.minimum(b + 1, NB - 1)
        for j in range(4):
            m2 = m_ref[par * 4 + j] if consume else None
            m_ref[(1 - par) * 4 + j] = item(j, b1, sbufs[(1 - par) * 4 + j], b, sbufs[par * 4 + j], m2,
                                            (os0, os1)[par], True, consume)

    def a2_body(b, c):
        @pl.when(b % 2 == 0)
        def _():
            block(b, 0)

        @pl.when(b % 2 == 1)
        def _():
            block(b, 1)
        return c

    def last_block_units():
        b = NB - 1
        flush_o(b - 1, os0)
        for hh in range(4):
            sr = sbufs[4 + hh]
            m2 = m_ref[4 + hh]
            h2 = (b // NQB) * 4 + hh
            acc = l = None
            for kt in range(NKT):
                p, ll = probs(sr, kt, m2)
                l = ll if l is None else l + ll
                o = _dot(vt_tile(h2, kt), p)
                acc = o if acc is None else acc + o
                if kt == NKT - 1:
                    os1[hh * DA:(hh + 1) * DA, :] = acc * (1.0 / jnp.sum(l, axis=0, keepdims=True))
                yield
        flush_o(b, os1)

    t_flush(1, NQB - 1)
    block(-1, 1, consume=False)
    os1[...] = jnp.zeros(os1.shape, f32)
    lax.fori_loop(0, NB - 1, a2_body, 0)

    cp_woa.wait()
    cp_xb.wait()
    cp_wob.wait()
    scale = DB ** -0.5 * LOG2E
    h_ref[0:M, :] = mem0_ref[...].astype(f32)
    row = lax.broadcasted_iota(jnp.int32, (L, L), 0)
    col = lax.broadcasted_iota(jnp.int32, (L, L), 1)
    mask = (row < M) | (row >= col)

    def w(ref, r0, nr, c0, nc):
        return _up(ref[r0 // 2:(r0 + nr) // 2, c0:c0 + nc])

    def a4_part(s, p):
        prow = pl.ds(pl.multiple_of(s * (SEG // 2), SEG // 2), SEG // 2)
        o_ = jnp.concatenate([_up(oa[g, prow, :]) for g in range(8)], axis=1)
        wd = D // NAP
        y = _dot(o_, _up(woa[:, p * wd:(p + 1) * wd]))
        outa[pl.ds(pl.multiple_of(s * SEG, SEG), SEG), p * wd:(p + 1) * wd] = y.astype(bf16)

    def segment(s, order, s0, side=None):
        h_ref[M:L, :] = _up(xb[pl.ds(pl.multiple_of(s * (SEG // 2), SEG // 2), SEG // 2), :]).astype(f32)
        hv = h_ref[...]
        st = {}
        acc = {}
        for op, g, part in order:
            if op == 'U':
                next(side)
            elif op == 'A':
                a4_part(s0 + g // NAP, g % NAP)
            elif op in ('q', 'k', 'v'):
                ref = {'q': wq, 'k': wk, 'v': wv}[op]
                st[op, g] = _dot(hv, w(ref, 0, D, g * G * DB, G * DB))
            elif op == 'qk':
                q = st.pop(('q', g))
                k = st.pop(('k', g))
                st['s', g] = [
                    lax.dot_general(q[:, j * DB:(j + 1) * DB], k[:, j * DB:(j + 1) * DB].astype(bf16),
                                    (((1,), (1,)), ((), ())), preferred_element_type=f32)
                    for j in range(G)]
            elif op == 'sm':
                ps = []
                for sc in st.pop(('s', g)):
                    sc = jnp.where(mask, sc * scale, -1e9)
                    p = jnp.exp2(sc - jnp.max(sc, axis=-1, keepdims=True))
                    ps.append(p / jnp.sum(p, axis=-1, keepdims=True))
                st['p', g] = ps
            elif op == 'pv':
                v = st.pop(('v', g))
                st['ov', g] = jnp.concatenate(
                    [_dot(p, v[:, j * DB:(j + 1) * DB].astype(bf16))
                     for j, p in enumerate(st.pop(('p', g)))], axis=1)
            elif op == 'o':
                hf = 'ab'.index(part)
                r = _dot(st['ov', g], w(wob, g * G * DB, G * DB, hf * (D // 2), D // 2))
                acc[hf] = r if hf not in acc else acc[hf] + r
        for hf in (0, 1):
            cols = slice(hf * (D // 2), (hf + 1) * (D // 2))
            h_ref[0:M, cols] = acc[hf][0:M, :].astype(bf16).astype(f32)
            outb[pl.ds(pl.multiple_of(s * SEG, SEG), SEG), cols] = acc[hf][M:L, :].astype(bf16)

    def out_start(i):
        rows = pl.ds(i * (UNROLL * SEG), UNROLL * SEG)
        pltpu.make_async_copy(outa.at[rows, :], out_hbm.at[rows, pl.ds(0, D)], osems.at[0]).start()
        pltpu.make_async_copy(outb.at[rows, :], out_hbm.at[rows, pl.ds(D, D)], osems.at[1]).start()

    side = last_block_units()
    for u in range(UNROLL):
        segment(u, _parse_order(B_FIRST[u]), 0, side)
    for _ in side:
        pass
    out_start(0)

    orders = [_parse_order(t) for t in B_ORDER]

    def b_body(i, c):
        for u in range(UNROLL):
            segment(i * UNROLL + u, orders[u], i * UNROLL)
        out_start(i)
        return c

    lax.fori_loop(1, NSEG // UNROLL, b_body, 0)

    pltpu.make_async_copy(outa, out_hbm.at[:, pl.ds(0, D)], osems.at[0]).wait()
    pltpu.make_async_copy(outb, out_hbm.at[:, pl.ds(D, D)], osems.at[1]).wait()


@functools.partial(jax.jit, static_argnames=("B_seg_len",))
def pallas_concat_heads__softmax_full_mha__memory_aug_recurrent_mem_tr__prompt_kernel(
        A_x, A_wqkv, A_wo, B_x, B_mem0, B_Wq, B_Wk, B_Wv, B_Wo, B_seg_len):
    assert B_seg_len == SEG and A_x.shape == (1, S, D) and B_x.shape == (1, S, D)
    assert B_mem0.shape == (1, M, D) and B_Wq.shape == (D, HB, DB) and B_Wo.shape == (HB, DB, D)
    hbm = pl.BlockSpec(memory_space=pl.ANY)
    V = pltpu.VMEM
    scratch = [
        V((S // 2, D), u32),
        V((D // 2, 3 * D), u32),
        V((D // 2, D), u32),
        V((8, S // 2, 128), u32),
        V((2, NQB, HA, DA // 2, QB), u32),
        V((QB // 2, D), u32),
        V((8, S // 2, 128), u32),
    ] + [V((S, QB), f32) for _ in range(8)] + [
        V((8, 1, QB), f32),
        V((128, QB), f32), V((128, QB), f32),
        V((D // 2, HB * DB), u32),
        V((D // 2, HB * DB), u32),
        V((D // 2, HB * DB), u32),
        V((HB * DB // 2, D), u32),
        V((S // 2, D), u32),
        V((NSLOT, 3, RC * 256, 128), u32),
        V((S, D), bf16),
        V((S, D), bf16),
        V((L, D), f32),
        V((8, 128), u32),
        pltpu.SemaphoreType.DMA((14,)),
        pltpu.SemaphoreType.DMA((NSLOT, 3)),
        pltpu.SemaphoreType.DMA((2,)),
    ]
    out = pl.pallas_call(
        _kernel,
        out_shape=jax.ShapeDtypeStruct((S, 2 * D), bf16),
        in_specs=[hbm, hbm, hbm, hbm, pl.BlockSpec(memory_space=pltpu.VMEM), hbm, hbm, hbm, hbm],
        out_specs=hbm,
        scratch_shapes=scratch,
        compiler_params=pltpu.CompilerParams(vmem_limit_bytes=120 * 1024 * 1024),
    )(A_x.reshape(S, D), A_wqkv, A_wo, B_x.reshape(S, D), B_mem0.reshape(M, D),
      B_Wq.reshape(D * HB, DB), B_Wk.reshape(D * HB, DB), B_Wv.reshape(D * HB, DB),
      B_Wo.reshape(HB * DB, D))
    return out.reshape(1, S, 2 * D)
```

```python
import functools
import math

import jax
import jax.numpy as jnp
from jax import lax
import jax.experimental.pallas as pl
import jax.experimental.pallas.tpu as pltpu

bf16 = jnp.bfloat16
f32 = jnp.float32
u32 = jnp.uint32

S = 2048
D = 1024
HA, DA = 32, 32
HB, DB = 32, 128
M, SEG = 8, 32
L = M + SEG
NSEG = S // SEG

QB = 512
QP = QB // 2
NQB = S // QB
KT = 128
NKT = S // KT
NB = HA * NQB // 4
TREE = 4

G = 4
UNROLL = 2
NAP = 2

NWC = 4
WC = D // NWC
RC = 8
NRC = D // 16 // RC
NSLOT = 3

LOG2E = math.log2(math.e)

B_ORDER = (
    ('k0 q0 q1 v0 qk0 sm0 k1 q2 qk1 pv0 sm1 v1 k2 o0b pv1 v2 qk2 o0a o1b A3 sm2 q3 pv2 k3 o1a qk3 '
     'o2a sm3 v3 q4 pv3 k4 v4 qk4 o2b o3b o3a sm4 q5 pv4 k5 o4a qk5 v5 o4b sm5 q6 pv5 k6 o5a k7 '
     'qk6 A2 sm6 v6 q7 o5b qk7 sm7 pv6 v7 o6a pv7 o6b o7a o7b A0 '),
    ('q0 k0 q1 qk0 v0 sm0 k1 q2 pv0 o0b qk1 A1 v1 sm1 k2 pv1 v2 o1b qk2 sm2 q3 o0a o1a pv2 k3 o2a '
     'qk3 v3 q4 sm3 pv3 k4 o2b o3b qk4 sm4 o3a v4 q5 pv4 k5 v5 o4a o4b qk5 k6 q6 sm5 pv5 k7 qk6 '
     'o5a sm6 v6 q7 pv6 o5b qk7 v7 sm7 o6a pv7 o6b o7b o7a '),
)
B_FIRST = (
    ('U k0 q0 q1 U v0 U qk0 sm0 U k1 q2 U qk1 U sm1 pv0 v1 k2 U pv1 A1 o0b U v2 U o0a qk2 U o1b A3 '
     'U q3 sm2 k3 U pv2 U qk3 U sm3 o2a o1a U A2 U v3 pv3 o2b k4 q4 v4 qk4 U U o3a U o3b sm4 U q5 '
     'pv4 k5 o4a U qk5 U o4b v5 sm5 U q6 pv5 k6 U U k7 qk6 U o5a sm6 v6 U q7 U U pv6 o5b qk7 U v7 '
     'sm7 o6a A0 U pv7 o6b U o7a o7b U U '),
    ('q0 U U k0 q1 qk0 U v0 U k1 q2 U sm0 pv0 o0b qk1 U sm1 U v1 U k2 pv1 U v2 o1b U qk2 sm2 q3 U '
     'o0a o1a U pv2 U k3 o2a U U qk3 v3 q4 sm3 U pv3 k4 U o2b o3b U qk4 sm4 U o3a v4 U q5 pv4 U k5 '
     'v5 U o4a o4b U qk5 k6 U q6 sm5 pv5 U k7 U qk6 U U v6 o5b q7 sm6 pv6 o5a U qk7 U sm7 v7 o6a '
     'pv7 o6b o7b o7a '),
)


def _parse_order(txt):
    out = []
    for t in txt.split():
        if t == 'U':
            out.append(('U', 0, ''))
            continue
        part = t[-1] if t[-1] in 'ab' else ''
        t = t[:-1] if part else t
        out.append((t[:-1], int(t[-1]), part))
    return out


def _pk(x):
    return pltpu.bitcast(x, u32)


def _up(x):
    return pltpu.bitcast(x, bf16)


def _dot(a, b):
    return jnp.dot(a, b, preferred_element_type=f32)


def _kernel(xa_hbm, wqkv_hbm, woa_hbm, xb_hbm, mem0_ref, wq_hbm, wk_hbm, wv_hbm, wob_hbm,
            out_hbm,
            xa, wqkv, woa, k3, qvt, tstage, oa, s0, s1, s2, s3, s4, s5, s6, s7, m_ref, os0, os1,
            wq, wk, wv, wob, xb, raw, outa, outb, h_ref, z_ref, sems, rsems, osems):
    qt = qvt.at[0]
    vt = qvt.at[1]
    z_ref[...] = jnp.zeros(z_ref.shape, u32)

    xa32 = xa_hbm.bitcast(u32)
    wqkv32 = wqkv_hbm.bitcast(u32)

    def cp_x0(hf):
        rows = pl.ds(hf * (QP // 2), QP // 2)
        return pltpu.make_async_copy(xa32.at[rows, :], xa.at[rows, :], sems.at[(0, 13)[hf]])

    def cp_xa(r):
        rows = pl.ds(r * QP, QP)
        return pltpu.make_async_copy(xa32.at[rows, :], xa.at[rows, :], sems.at[r])

    def cp_wq(c):
        cols = pl.ds(c * WC, WC)
        return pltpu.make_async_copy(wqkv32.at[:, cols], wqkv.at[:, cols], sems.at[4 + c])

    def cp_wkv(i):
        cols = pl.ds(i * D, D)
        return pltpu.make_async_copy(wqkv32.at[:, cols], wqkv.at[:, cols], sems.at[7 + i])

    cp_woa = pltpu.make_async_copy(woa_hbm.bitcast(u32), woa, sems.at[10])
    cp_xb = pltpu.make_async_copy(xb_hbm.bitcast(u32), xb, sems.at[11])
    cp_wob = pltpu.make_async_copy(wob_hbm.bitcast(u32), wob, sems.at[12])

    w_hbms = (wq_hbm, wk_hbm, wv_hbm)
    w_dsts = (wq, wk, wv)

    def raw_copy(c, i):
        return pltpu.make_async_copy(
            w_hbms[i].bitcast(u32).at[pl.ds(c * (RC * 256), RC * 256), :],
            raw.at[c % NSLOT, i], rsems.at[c % NSLOT, i])

    def raw_start(c):
        for i in range(3):
            raw_copy(c, i).start()

    def raw_step(c):
        for i in range(3):
            raw_copy(c, i).wait()

        @pl.when(c + NSLOT - 1 < NRC)
        def _():
            raw_start(c + NSLOT - 1)

    def relayout_chunk(c):
        slot = c % NSLOT
        z = z_ref[...]
        hm = jnp.uint32(0xFFFF0000)
        prev = None
        for t in range(RC):
            rows = pl.ds(pl.multiple_of((c * RC + t) * 8, 8), 8)
            for i in range(3):
                for j in range(HB // 2):
                    a = raw[slot, i, pl.ds(t * 256 + j, 8, stride=16), :]
                    b = raw[slot, i, pl.ds(t * 256 + 128 + j, 8, stride=16), :]
                    if prev is not None:
                        pz = prev & z
                        a = a | pz
                        b = b | pz
                    lo = jnp.concatenate([pltpu.bitcast(a << 16, f32), pltpu.bitcast(b << 16, f32)], axis=0)
                    hi = jnp.concatenate([pltpu.bitcast(a & hm, f32), pltpu.bitcast(b & hm, f32)], axis=0)
                    lo = _pk(lo.astype(bf16))
                    hi = _pk(hi.astype(bf16))
                    w_dsts[i][rows, (2 * j) * DB:(2 * j + 1) * DB] = lo
                    w_dsts[i][rows, (2 * j + 1) * DB:(2 * j + 2) * DB] = hi
                    prev = hi

    qscale = DA ** -0.5 * LOG2E

    def xrows(r):
        return _up(xa[pl.ds(pl.multiple_of(r * QP, QP), QP), :])

    def q_dot(x_, c0, nc):
        return _dot(x_, _up(wqkv[:, c0:c0 + nc])) * qscale

    def t_stage(y, r0, c0):
        tstage[r0 // 2:(r0 + y.shape[0]) // 2, c0:c0 + y.shape[1]] = _pk(y.astype(bf16))

    def t_flush(which, r):
        for g in range(8):
            t = _up(tstage[:, g * 128:(g + 1) * 128]).astype(f32).T.astype(bf16)
            qvt[which, r, g * 4:g * 4 + 4] = _pk(t).reshape(4, DA // 2, QB)

    def a1_q(r, c):
        cp_xa(r).wait()
        t_flush(0, r - 1)
        t_stage(q_dot(xrows(r), 0, D), 0, 0)
        return c

    def a1_k(r, c):
        raw_step(r)
        k = _dot(xrows(r), _up(wqkv[:, D:2 * D])).astype(bf16)
        for g in range(8):
            k3[g, pl.ds(pl.multiple_of(r * QP, QP), QP), :] = _pk(k[:, g * 128:(g + 1) * 128])
        relayout_chunk(r)
        return c

    def a1_v(r, c):
        raw_step(NQB + r)
        t_flush(jnp.where(r == 0, 0, 1), jnp.where(r == 0, NQB - 1, r - 1))
        t_stage(_dot(xrows(r), _up(wqkv[:, 2 * D:3 * D])), 0, 0)
        relayout_chunk(NQB + r)
        return c

    cp_wq(0).start()
    cp_x0(0).start()
    cp_x0(1).start()
    for c in range(1, NWC):
        cp_wq(c).start()
    for r in range(1, NQB):
        cp_xa(r).start()
    cp_wkv(1).start()
    raw_start(0)
    cp_wkv(2).start()
    for c in range(1, NSLOT - 1):
        raw_start(c)

    def x0half(hf):
        return _up(xa[hf * (QP // 2):(hf + 1) * (QP // 2), :])

    pieces = [(cp_x0(0), lambda: x0half(0), 0, 0), (cp_x0(1), lambda: x0half(1), QB // 2, 0)]
    pieces += [(cp_wq(c), lambda: xrows(0), 0, c * WC) for c in range(1, NWC)]
    cp_wq(0).wait()
    prev = None
    for cp, lhs, r0, c0 in pieces:
        cp.wait()
        y = q_dot(lhs(), c0, WC)
        if prev is not None:
            t_stage(*prev)
        prev = (y, r0, c0)
    t_stage(*prev)

    lax.fori_loop(1, NQB, a1_q, 0)
    cp_wkv(1).wait()
    lax.fori_loop(0, NQB, a1_k, 0)
    cp_wkv(2).wait()
    lax.fori_loop(0, NQB, a1_v, 0)
    cp_woa.start()
    cp_xb.start()
    cp_wob.start()

    sbufs = (s0, s1, s2, s3, s4, s5, s6, s7)

    def probs(sr, kt, m2):
        p = jnp.exp2(sr[kt * KT:(kt + 1) * KT, :] - m2)
        t = p.reshape(KT // 8, 8, QB)
        for _ in range(TREE):
            t4 = t.reshape(t.shape[0] // 2, 2, 8, QB)
            t = t4[:, 0] + t4[:, 1]
        return p.astype(bf16), jnp.sum(t, axis=0)

    def vt_tile(h, kt):
        r_, c_ = divmod(kt * KT, QB)
        return _up(vt[r_, h, :, c_:c_ + KT])

    def item(hh, b1, sw, b2, sr, m2, ostage, produce, consume):
        m = acc = l = None
        if produce:
            g1 = b1 // NQB
            parts = []
            if hh > 0:
                parts.append(jnp.zeros((DA * hh, QB), bf16))
            parts.append(_up(qt[b1 % NQB, g1 * 4 + hh]))
            if hh < 3:
                parts.append(jnp.zeros((DA * (3 - hh), QB), bf16))
            q_ = jnp.concatenate(parts, axis=0)
        if consume:
            h2 = (b2 // NQB) * 4 + hh
        for kt in range(NKT):
            if produce:
                st = _dot(_up(k3[g1, kt * (KT // 2):(kt + 1) * (KT // 2), :]), q_)
                sw[kt * KT:(kt + 1) * KT, :] = st
                mm = jnp.max(st.reshape(KT // 8, 8, QB), axis=0)
                m = mm if m is None else jnp.maximum(m, mm)
            if consume:
                p, ll = probs(sr, kt, m2)
                l = ll if l is None else l + ll
                o = _dot(vt_tile(h2, kt), p)
                acc = o if acc is None else acc + o
        if consume:
            ostage[hh * DA:(hh + 1) * DA, :] = acc * (1.0 / jnp.sum(l, axis=0, keepdims=True))
        if produce:
            return jnp.max(m, axis=0, keepdims=True)

    def flush_o(b, ostage):
        b = jnp.maximum(b, 0)
        oa[b // NQB, pl.ds(pl.multiple_of((b % NQB) * QP, QP), QP), :] = _pk(ostage[...].T.astype(bf16))

    def block(b, par, consume=True):
        if consume:
            flush_o(b - 1, (os0, os1)[1 - par])
        b1 = jnp.minimum(b + 1, NB - 1)
        for j in range(4):
            m2 = m_ref[par * 4 + j] if consume else None
            m_ref[(1 - par) * 4 + j] = item(j, b1, sbufs[(1 - par) * 4 + j], b, sbufs[par * 4 + j], m2,
                                            (os0, os1)[par], True, consume)

    def a2_body(b, c):
        @pl.when(b % 2 == 0)
        def _():
            block(b, 0)

        @pl.when(b % 2 == 1)
        def _():
            block(b, 1)
        return c

    def last_block_units():
        b = NB - 1
        flush_o(b - 1, os0)
        for hh in range(4):
            sr = sbufs[4 + hh]
            m2 = m_ref[4 + hh]
            h2 = (b // NQB) * 4 + hh
            acc = l = None
            for kt in range(NKT):
                p, ll = probs(sr, kt, m2)
                l = ll if l is None else l + ll
                o = _dot(vt_tile(h2, kt), p)
                acc = o if acc is None else acc + o
                if kt == NKT - 1:
                    os1[hh * DA:(hh + 1) * DA, :] = acc * (1.0 / jnp.sum(l, axis=0, keepdims=True))
                yield
        flush_o(b, os1)

    t_flush(1, NQB - 1)
    block(-1, 1, consume=False)
    os1[...] = jnp.zeros(os1.shape, f32)
    lax.fori_loop(0, NB - 1, a2_body, 0)

    cp_woa.wait()
    cp_xb.wait()
    cp_wob.wait()
    scale = DB ** -0.5 * LOG2E
    h_ref[0:M, :] = mem0_ref[...].astype(f32)
    row = lax.broadcasted_iota(jnp.int32, (L, L), 0)
    col = lax.broadcasted_iota(jnp.int32, (L, L), 1)
    mask = (row < M) | (row >= col)

    def w(ref, r0, nr, c0, nc):
        return _up(ref[r0 // 2:(r0 + nr) // 2, c0:c0 + nc])

    def a4_part(s, p):
        prow = pl.ds(pl.multiple_of(s * (SEG // 2), SEG // 2), SEG // 2)
        o_ = jnp.concatenate([_up(oa[g, prow, :]) for g in range(8)], axis=1)
        wd = D // NAP
        y = _dot(o_, _up(woa[:, p * wd:(p + 1) * wd]))
        outa[pl.ds(pl.multiple_of(s * SEG, SEG), SEG), p * wd:(p + 1) * wd] = y.astype(bf16)

    def segment(s, order, s0, side=None):
        h_ref[M:L, :] = _up(xb[pl.ds(pl.multiple_of(s * (SEG // 2), SEG // 2), SEG // 2), :]).astype(f32)
        hv = h_ref[...]
        st = {}
        acc = {}
        for op, g, part in order:
            if op == 'U':
                next(side)
            elif op == 'A':
                a4_part(s0 + g // NAP, g % NAP)
            elif op in ('q', 'k', 'v'):
                ref = {'q': wq, 'k': wk, 'v': wv}[op]
                st[op, g] = _dot(hv, w(ref, 0, D, g * G * DB, G * DB))
            elif op == 'qk':
                q = st.pop(('q', g))
                k = st.pop(('k', g))
                st['s', g] = [
                    lax.dot_general(q[:, j * DB:(j + 1) * DB], k[:, j * DB:(j + 1) * DB].astype(bf16),
                                    (((1,), (1,)), ((), ())), preferred_element_type=f32)
                    for j in range(G)]
            elif op == 'sm':
                ps = []
                for sc in st.pop(('s', g)):
                    sc = jnp.where(mask, sc * scale, -1e9)
                    p = jnp.exp2(sc - jnp.max(sc, axis=-1, keepdims=True))
                    ps.append(p / jnp.sum(p, axis=-1, keepdims=True))
                st['p', g] = ps
            elif op == 'pv':
                v = st.pop(('v', g))
                st['ov', g] = jnp.concatenate(
                    [_dot(p, v[:, j * DB:(j + 1) * DB].astype(bf16))
                     for j, p in enumerate(st.pop(('p', g)))], axis=1)
            elif op == 'o':
                hf = 'ab'.index(part)
                r = _dot(st['ov', g], w(wob, g * G * DB, G * DB, hf * (D // 2), D // 2))
                acc[hf] = r if hf not in acc else acc[hf] + r
        for hf in (0, 1):
            cols = slice(hf * (D // 2), (hf + 1) * (D // 2))
            h_ref[0:M, cols] = acc[hf][0:M, :].astype(bf16).astype(f32)
            outb[pl.ds(pl.multiple_of(s * SEG, SEG), SEG), cols] = acc[hf][M:L, :].astype(bf16)

    def out_start(i):
        rows = pl.ds(i * (UNROLL * SEG), UNROLL * SEG)
        pltpu.make_async_copy(outa.at[rows, :], out_hbm.at[rows, pl.ds(0, D)], osems.at[0]).start()
        pltpu.make_async_copy(outb.at[rows, :], out_hbm.at[rows, pl.ds(D, D)], osems.at[1]).start()

    side = last_block_units()
    for u in range(UNROLL):
        segment(u, _parse_order(B_FIRST[u]), 0, side)
    for _ in side:
        pass
    out_start(0)

    orders = [_parse_order(t) for t in B_ORDER]

    def b_body(i, c):
        for u in range(UNROLL):
            segment(i * UNROLL + u, orders[u], i * UNROLL)
        out_start(i)
        return c

    lax.fori_loop(1, NSEG // UNROLL, b_body, 0)

    pltpu.make_async_copy(outa, out_hbm.at[:, pl.ds(0, D)], osems.at[0]).wait()
    pltpu.make_async_copy(outb, out_hbm.at[:, pl.ds(D, D)], osems.at[1]).wait()


@functools.partial(jax.jit, static_argnames=("B_seg_len",))
def pallas_concat_heads__softmax_full_mha__memory_aug_recurrent_mem_tr__prompt_kernel(
        A_x, A_wqkv, A_wo, B_x, B_mem0, B_Wq, B_Wk, B_Wv, B_Wo, B_seg_len):
    assert B_seg_len == SEG and A_x.shape == (1, S, D) and B_x.shape == (1, S, D)
    assert B_mem0.shape == (1, M, D) and B_Wq.shape == (D, HB, DB) and B_Wo.shape == (HB, DB, D)
    hbm = pl.BlockSpec(memory_space=pl.ANY)
    V = pltpu.VMEM
    scratch = [
        V((S // 2, D), u32),
        V((D // 2, 3 * D), u32),
        V((D // 2, D), u32),
        V((8, S // 2, 128), u32),
        V((2, NQB, HA, DA // 2, QB), u32),
        V((QB // 2, D), u32),
        V((8, S // 2, 128), u32),
    ] + [V((S, QB), f32) for _ in range(8)] + [
        V((8, 1, QB), f32),
        V((128, QB), f32), V((128, QB), f32),
        V((D // 2, HB * DB), u32),
        V((D // 2, HB * DB), u32),
        V((D // 2, HB * DB), u32),
        V((HB * DB // 2, D), u32),
        V((S // 2, D), u32),
        V((NSLOT, 3, RC * 256, 128), u32),
        V((S, D), bf16),
        V((S, D), bf16),
        V((L, D), f32),
        V((8, 128), u32),
        pltpu.SemaphoreType.DMA((14,)),
        pltpu.SemaphoreType.DMA((NSLOT, 3)),
        pltpu.SemaphoreType.DMA((2,)),
    ]
    out = pl.pallas_call(
        _kernel,
        out_shape=jax.ShapeDtypeStruct((S, 2 * D), bf16),
        in_specs=[hbm, hbm, hbm, hbm, pl.BlockSpec(memory_space=pltpu.VMEM), hbm, hbm, hbm, hbm],
        out_specs=hbm,
        scratch_shapes=scratch,
        compiler_params=pltpu.CompilerParams(vmem_limit_bytes=120 * 1024 * 1024),
    )(A_x.reshape(S, D), A_wqkv, A_wo, B_x.reshape(S, D), B_mem0.reshape(M, D),
      B_Wq.reshape(D * HB, DB), B_Wk.reshape(D * HB, DB), B_Wv.reshape(D * HB, DB),
      B_Wo.reshape(HB * DB, D))
    return out.reshape(1, S, 2 * D)
```

```python
import functools
import math

import jax
import jax.numpy as jnp
from jax import lax
import jax.experimental.pallas as pl
import jax.experimental.pallas.tpu as pltpu

bf16 = jnp.bfloat16
f32 = jnp.float32
u32 = jnp.uint32

S = 2048
D = 1024
HA, DA = 32, 32
HB, DB = 32, 128
M, SEG = 8, 32
L = M + SEG
NSEG = S // SEG

QB = 512
QP = QB // 2
NQB = S // QB
KT = 128
NKT = S // KT
NB = HA * NQB // 4
TREE = 4

G = 4
UNROLL = 2
NAP = 2

NWC = 4
WC = D // NWC
RC = 8
NRC = D // 16 // RC
NSLOT = 3

LOG2E = math.log2(math.e)

B_ORDER = (
    ('k0 q0 q1 v0 qk0 sm0 k1 q2 qk1 pv0 sm1 v1 k2 o0b pv1 v2 qk2 o0a o1b A3 sm2 q3 pv2 k3 o1a qk3 '
     'o2a sm3 v3 q4 pv3 k4 v4 qk4 o2b o3b o3a sm4 q5 pv4 k5 o4a qk5 v5 o4b sm5 q6 pv5 k6 o5a k7 '
     'qk6 A2 sm6 v6 q7 o5b qk7 sm7 pv6 v7 o6a pv7 o6b o7a o7b A0 '),
    ('q0 k0 q1 qk0 v0 sm0 k1 q2 pv0 o0b qk1 A1 v1 sm1 k2 pv1 v2 o1b qk2 sm2 q3 o0a o1a pv2 k3 o2a '
     'qk3 v3 q4 sm3 pv3 k4 o2b o3b qk4 sm4 o3a v4 q5 pv4 k5 v5 o4a o4b qk5 k6 q6 sm5 pv5 k7 qk6 '
     'o5a sm6 v6 q7 pv6 o5b qk7 v7 sm7 o6a pv7 o6b o7b o7a '),
)
B_FIRST = (
    ('U k0 q0 q1 U v0 U qk0 sm0 U k1 q2 U qk1 U sm1 pv0 v1 k2 U pv1 A1 o0b U v2 U o0a qk2 U o1b A3 '
     'U q3 sm2 k3 U pv2 U qk3 U sm3 o2a o1a U A2 U v3 pv3 o2b k4 q4 v4 qk4 U U o3a U o3b sm4 U q5 '
     'pv4 k5 o4a U qk5 U o4b v5 sm5 U q6 pv5 k6 U U k7 qk6 U o5a sm6 v6 U q7 U U pv6 o5b qk7 U v7 '
     'sm7 o6a A0 U pv7 o6b U o7a o7b U U '),
    ('q0 U U k0 q1 qk0 U v0 U k1 q2 U sm0 pv0 o0b qk1 U sm1 U v1 U k2 pv1 U v2 o1b U qk2 sm2 q3 U '
     'o0a o1a U pv2 U k3 o2a U U qk3 v3 q4 sm3 U pv3 k4 U o2b o3b U qk4 sm4 U o3a v4 U q5 pv4 U k5 '
     'v5 U o4a o4b U qk5 k6 U q6 sm5 pv5 U k7 U qk6 U U v6 o5b q7 sm6 pv6 o5a U qk7 U sm7 v7 o6a '
     'pv7 o6b o7b o7a '),
)


def _parse_order(txt):
    out = []
    for t in txt.split():
        if t == 'U':
            out.append(('U', 0, ''))
            continue
        part = t[-1] if t[-1] in 'ab' else ''
        t = t[:-1] if part else t
        out.append((t[:-1], int(t[-1]), part))
    return out


def _pk(x):
    return pltpu.bitcast(x, u32)


def _up(x):
    return pltpu.bitcast(x, bf16)


def _dot(a, b):
    return jnp.dot(a, b, preferred_element_type=f32)


def _kernel(xa_hbm, wqkv_hbm, woa_hbm, xb_hbm, mem0_hbm, wq_hbm, wk_hbm, wv_hbm, wob_hbm,
            out_hbm,
            xa, wqkv, woa, k3, qvt, tstage, oa, s0, s1, s2, s3, s4, s5, s6, s7, m_ref, os0, os1,
            wq, wk, wv, wob, xb, raw, outa, outb, h_ref, mem0, z_ref, sems, rsems, osems):
    qt = qvt.at[0]
    vt = qvt.at[1]
    z_ref[...] = jnp.zeros(z_ref.shape, u32)

    xa32 = xa_hbm.bitcast(u32)
    wqkv32 = wqkv_hbm.bitcast(u32)

    def cp_x0(hf):
        rows = pl.ds(hf * (QP // 2), QP // 2)
        return pltpu.make_async_copy(xa32.at[rows, :], xa.at[rows, :], sems.at[(0, 13)[hf]])

    def cp_xa(r):
        rows = pl.ds(r * QP, QP)
        return pltpu.make_async_copy(xa32.at[rows, :], xa.at[rows, :], sems.at[r])

    def cp_wq(c):
        cols = pl.ds(c * WC, WC)
        return pltpu.make_async_copy(wqkv32.at[:, cols], wqkv.at[:, cols], sems.at[4 + c])

    def cp_wkv(i):
        cols = pl.ds(i * D, D)
        return pltpu.make_async_copy(wqkv32.at[:, cols], wqkv.at[:, cols], sems.at[7 + i])

    cp_woa = pltpu.make_async_copy(woa_hbm.bitcast(u32), woa, sems.at[10])
    cp_xb = pltpu.make_async_copy(xb_hbm.bitcast(u32), xb, sems.at[11])
    cp_wob = pltpu.make_async_copy(wob_hbm.bitcast(u32), wob, sems.at[12])
    cp_mem0 = pltpu.make_async_copy(mem0_hbm, mem0, sems.at[14])

    w_hbms = (wq_hbm, wk_hbm, wv_hbm)
    w_dsts = (wq, wk, wv)

    def raw_copy(c, i):
        return pltpu.make_async_copy(
            w_hbms[i].bitcast(u32).at[pl.ds(c * (RC * 256), RC * 256), :],
            raw.at[c % NSLOT, i], rsems.at[c % NSLOT, i])

    def raw_start(c):
        for i in range(3):
            raw_copy(c, i).start()

    def raw_step(c):
        for i in range(3):
            raw_copy(c, i).wait()

        @pl.when(c + NSLOT - 1 < NRC)
        def _():
            raw_start(c + NSLOT - 1)

    def relayout_chunk(c):
        slot = c % NSLOT
        z = z_ref[...]
        hm = jnp.uint32(0xFFFF0000)
        prev = None
        for t in range(RC):
            rows = pl.ds(pl.multiple_of((c * RC + t) * 8, 8), 8)
            for i in range(3):
                for j in range(HB // 2):
                    a = raw[slot, i, pl.ds(t * 256 + j, 8, stride=16), :]
                    b = raw[slot, i, pl.ds(t * 256 + 128 + j, 8, stride=16), :]
                    if prev is not None:
                        pz = prev & z
                        a = a | pz
                        b = b | pz
                    lo = jnp.concatenate([pltpu.bitcast(a << 16, f32), pltpu.bitcast(b << 16, f32)], axis=0)
                    hi = jnp.concatenate([pltpu.bitcast(a & hm, f32), pltpu.bitcast(b & hm, f32)], axis=0)
                    lo = _pk(lo.astype(bf16))
                    hi = _pk(hi.astype(bf16))
                    w_dsts[i][rows, (2 * j) * DB:(2 * j + 1) * DB] = lo
                    w_dsts[i][rows, (2 * j + 1) * DB:(2 * j + 2) * DB] = hi
                    prev = hi

    qscale = DA ** -0.5 * LOG2E

    def xrows(r):
        return _up(xa[pl.ds(pl.multiple_of(r * QP, QP), QP), :])

    def q_dot(x_, c0, nc):
        return _dot(x_, _up(wqkv[:, c0:c0 + nc])) * qscale

    def t_stage(y, r0, c0):
        tstage[r0 // 2:(r0 + y.shape[0]) // 2, c0:c0 + y.shape[1]] = _pk(y.astype(bf16))

    def t_flush(which, r):
        for g in range(8):
            t = _up(tstage[:, g * 128:(g + 1) * 128]).astype(f32).T.astype(bf16)
            qvt[which, r, g * 4:g * 4 + 4] = _pk(t).reshape(4, DA // 2, QB)

    def a1_q(r, c):
        cp_xa(r).wait()
        t_flush(0, r - 1)
        t_stage(q_dot(xrows(r), 0, D), 0, 0)
        return c

    def a1_k(r, c):
        raw_step(r)
        k = _dot(xrows(r), _up(wqkv[:, D:2 * D])).astype(bf16)
        for g in range(8):
            k3[g, pl.ds(pl.multiple_of(r * QP, QP), QP), :] = _pk(k[:, g * 128:(g + 1) * 128])
        relayout_chunk(r)
        return c

    def a1_v(r, c):
        raw_step(NQB + r)
        t_flush(jnp.where(r == 0, 0, 1), jnp.where(r == 0, NQB - 1, r - 1))
        t_stage(_dot(xrows(r), _up(wqkv[:, 2 * D:3 * D])), 0, 0)
        relayout_chunk(NQB + r)
        return c

    cp_wq(0).start()
    cp_x0(0).start()
    cp_x0(1).start()
    for c in range(1, NWC):
        cp_wq(c).start()
    for r in range(1, NQB):
        cp_xa(r).start()
    cp_wkv(1).start()
    raw_start(0)
    cp_wkv(2).start()
    for c in range(1, NSLOT - 1):
        raw_start(c)

    def x0half(hf):
        return _up(xa[hf * (QP // 2):(hf + 1) * (QP // 2), :])

    pieces = [(cp_x0(0), lambda: x0half(0), 0, 0), (cp_x0(1), lambda: x0half(1), QB // 2, 0)]
    pieces += [(cp_wq(c), lambda: xrows(0), 0, c * WC) for c in range(1, NWC)]
    cp_wq(0).wait()
    prev = None
    for cp, lhs, r0, c0 in pieces:
        cp.wait()
        y = q_dot(lhs(), c0, WC)
        if prev is not None:
            t_stage(*prev)
        prev = (y, r0, c0)
    t_stage(*prev)

    lax.fori_loop(1, NQB, a1_q, 0)
    cp_wkv(1).wait()
    lax.fori_loop(0, NQB, a1_k, 0)
    cp_wkv(2).wait()
    lax.fori_loop(0, NQB, a1_v, 0)
    cp_woa.start()
    cp_xb.start()
    cp_wob.start()
    cp_mem0.start()

    sbufs = (s0, s1, s2, s3, s4, s5, s6, s7)

    def probs(sr, kt, m2):
        p = jnp.exp2(sr[kt * KT:(kt + 1) * KT, :] - m2)
        t = p.reshape(KT // 8, 8, QB)
        for _ in range(TREE):
            t4 = t.reshape(t.shape[0] // 2, 2, 8, QB)
            t = t4[:, 0] + t4[:, 1]
        return p.astype(bf16), jnp.sum(t, axis=0)

    def vt_tile(h, kt):
        r_, c_ = divmod(kt * KT, QB)
        return _up(vt[r_, h, :, c_:c_ + KT])

    def item(hh, b1, sw, b2, sr, m2, ostage, produce, consume):
        m = acc = l = None
        if produce:
            g1 = b1 // NQB
            parts = []
            if hh > 0:
                parts.append(jnp.zeros((DA * hh, QB), bf16))
            parts.append(_up(qt[b1 % NQB, g1 * 4 + hh]))
            if hh < 3:
                parts.append(jnp.zeros((DA * (3 - hh), QB), bf16))
            q_ = jnp.concatenate(parts, axis=0)
        if consume:
            h2 = (b2 // NQB) * 4 + hh
        for kt in range(NKT):
            if produce:
                st = _dot(_up(k3[g1, kt * (KT // 2):(kt + 1) * (KT // 2), :]), q_)
                sw[kt * KT:(kt + 1) * KT, :] = st
                mm = jnp.max(st.reshape(KT // 8, 8, QB), axis=0)
                m = mm if m is None else jnp.maximum(m, mm)
            if consume:
                p, ll = probs(sr, kt, m2)
                l = ll if l is None else l + ll
                o = _dot(vt_tile(h2, kt), p)
                acc = o if acc is None else acc + o
        if consume:
            ostage[hh * DA:(hh + 1) * DA, :] = acc * (1.0 / jnp.sum(l, axis=0, keepdims=True))
        if produce:
            return jnp.max(m, axis=0, keepdims=True)

    def flush_o(b, ostage):
        b = jnp.maximum(b, 0)
        oa[b // NQB, pl.ds(pl.multiple_of((b % NQB) * QP, QP), QP), :] = _pk(ostage[...].T.astype(bf16))

    def block(b, par, consume=True):
        if consume:
            flush_o(b - 1, (os0, os1)[1 - par])
        b1 = jnp.minimum(b + 1, NB - 1)
        for j in range(4):
            m2 = m_ref[par * 4 + j] if consume else None
            m_ref[(1 - par) * 4 + j] = item(j, b1, sbufs[(1 - par) * 4 + j], b, sbufs[par * 4 + j], m2,
                                            (os0, os1)[par], True, consume)

    def a2_body(b, c):
        @pl.when(b % 2 == 0)
        def _():
            block(b, 0)

        @pl.when(b % 2 == 1)
        def _():
            block(b, 1)
        return c

    def last_block_units():
        b = NB - 1
        flush_o(b - 1, os0)
        for hh in range(4):
            sr = sbufs[4 + hh]
            m2 = m_ref[4 + hh]
            h2 = (b // NQB) * 4 + hh
            acc = l = None
            for kt in range(NKT):
                p, ll = probs(sr, kt, m2)
                l = ll if l is None else l + ll
                o = _dot(vt_tile(h2, kt), p)
                acc = o if acc is None else acc + o
                if kt == NKT - 1:
                    os1[hh * DA:(hh + 1) * DA, :] = acc * (1.0 / jnp.sum(l, axis=0, keepdims=True))
                yield
        flush_o(b, os1)

    t_flush(1, NQB - 1)
    block(-1, 1, consume=False)
    os1[...] = jnp.zeros(os1.shape, f32)
    lax.fori_loop(0, NB - 1, a2_body, 0)

    cp_woa.wait()
    cp_xb.wait()
    cp_wob.wait()
    cp_mem0.wait()
    scale = DB ** -0.5 * LOG2E
    h_ref[0:M, :] = mem0[...].astype(f32)
    row = lax.broadcasted_iota(jnp.int32, (L, L), 0)
    col = lax.broadcasted_iota(jnp.int32, (L, L), 1)
    mask = (row < M) | (row >= col)

    def w(ref, r0, nr, c0, nc):
        return _up(ref[r0 // 2:(r0 + nr) // 2, c0:c0 + nc])

    def a4_part(s, p):
        prow = pl.ds(pl.multiple_of(s * (SEG // 2), SEG // 2), SEG // 2)
        o_ = jnp.concatenate([_up(oa[g, prow, :]) for g in range(8)], axis=1)
        wd = D // NAP
        y = _dot(o_, _up(woa[:, p * wd:(p + 1) * wd]))
        outa[pl.ds(pl.multiple_of(s * SEG, SEG), SEG), p * wd:(p + 1) * wd] = y.astype(bf16)

    def segment(s, order, s0, side=None):
        h_ref[M:L, :] = _up(xb[pl.ds(pl.multiple_of(s * (SEG // 2), SEG // 2), SEG // 2), :]).astype(f32)
        hv = h_ref[...]
        st = {}
        acc = {}
        for op, g, part in order:
            if op == 'U':
                next(side)
            elif op == 'A':
                a4_part(s0 + g // NAP, g % NAP)
            elif op in ('q', 'k', 'v'):
                ref = {'q': wq, 'k': wk, 'v': wv}[op]
                st[op, g] = _dot(hv, w(ref, 0, D, g * G * DB, G * DB))
            elif op == 'qk':
                q = st.pop(('q', g))
                k = st.pop(('k', g))
                st['s', g] = [
                    lax.dot_general(q[:, j * DB:(j + 1) * DB], k[:, j * DB:(j + 1) * DB].astype(bf16),
                                    (((1,), (1,)), ((), ())), preferred_element_type=f32)
                    for j in range(G)]
            elif op == 'sm':
                ps = []
                for sc in st.pop(('s', g)):
                    sc = jnp.where(mask, sc * scale, -1e9)
                    p = jnp.exp2(sc - jnp.max(sc, axis=-1, keepdims=True))
                    ps.append(p / jnp.sum(p, axis=-1, keepdims=True))
                st['p', g] = ps
            elif op == 'pv':
                v = st.pop(('v', g))
                st['ov', g] = jnp.concatenate(
                    [_dot(p, v[:, j * DB:(j + 1) * DB].astype(bf16))
                     for j, p in enumerate(st.pop(('p', g)))], axis=1)
            elif op == 'o':
                hf = 'ab'.index(part)
                r = _dot(st['ov', g], w(wob, g * G * DB, G * DB, hf * (D // 2), D // 2))
                acc[hf] = r if hf not in acc else acc[hf] + r
        for hf in (0, 1):
            cols = slice(hf * (D // 2), (hf + 1) * (D // 2))
            h_ref[0:M, cols] = acc[hf][0:M, :].astype(bf16).astype(f32)
            outb[pl.ds(pl.multiple_of(s * SEG, SEG), SEG), cols] = acc[hf][M:L, :].astype(bf16)

    def out_start(i):
        rows = pl.ds(i * (UNROLL * SEG), UNROLL * SEG)
        pltpu.make_async_copy(outa.at[rows, :], out_hbm.at[rows, pl.ds(0, D)], osems.at[0]).start()
        pltpu.make_async_copy(outb.at[rows, :], out_hbm.at[rows, pl.ds(D, D)], osems.at[1]).start()

    side = last_block_units()
    for u in range(UNROLL):
        segment(u, _parse_order(B_FIRST[u]), 0, side)
    for _ in side:
        pass
    out_start(0)

    orders = [_parse_order(t) for t in B_ORDER]

    def b_body(i, c):
        for u in range(UNROLL):
            segment(i * UNROLL + u, orders[u], i * UNROLL)
        out_start(i)
        return c

    lax.fori_loop(1, NSEG // UNROLL, b_body, 0)

    pltpu.make_async_copy(outa, out_hbm.at[:, pl.ds(0, D)], osems.at[0]).wait()
    pltpu.make_async_copy(outb, out_hbm.at[:, pl.ds(D, D)], osems.at[1]).wait()


@functools.partial(jax.jit, static_argnames=("B_seg_len",))
def pallas_concat_heads__softmax_full_mha__memory_aug_recurrent_mem_tr__prompt_kernel(
        A_x, A_wqkv, A_wo, B_x, B_mem0, B_Wq, B_Wk, B_Wv, B_Wo, B_seg_len):
    assert B_seg_len == SEG and A_x.shape == (1, S, D) and B_x.shape == (1, S, D)
    assert B_mem0.shape == (1, M, D) and B_Wq.shape == (D, HB, DB) and B_Wo.shape == (HB, DB, D)
    hbm = pl.BlockSpec(memory_space=pl.ANY)
    V = pltpu.VMEM
    scratch = [
        V((S // 2, D), u32),
        V((D // 2, 3 * D), u32),
        V((D // 2, D), u32),
        V((8, S // 2, 128), u32),
        V((2, NQB, HA, DA // 2, QB), u32),
        V((QB // 2, D), u32),
        V((8, S // 2, 128), u32),
    ] + [V((S, QB), f32) for _ in range(8)] + [
        V((8, 1, QB), f32),
        V((128, QB), f32), V((128, QB), f32),
        V((D // 2, HB * DB), u32),
        V((D // 2, HB * DB), u32),
        V((D // 2, HB * DB), u32),
        V((HB * DB // 2, D), u32),
        V((S // 2, D), u32),
        V((NSLOT, 3, RC * 256, 128), u32),
        V((S, D), bf16),
        V((S, D), bf16),
        V((L, D), f32),
        V((M, D), bf16),
        V((8, 128), u32),
        pltpu.SemaphoreType.DMA((15,)),
        pltpu.SemaphoreType.DMA((NSLOT, 3)),
        pltpu.SemaphoreType.DMA((2,)),
    ]
    out = pl.pallas_call(
        _kernel,
        out_shape=jax.ShapeDtypeStruct((S, 2 * D), bf16),
        in_specs=[hbm] * 9,
        out_specs=hbm,
        scratch_shapes=scratch,
        compiler_params=pltpu.CompilerParams(vmem_limit_bytes=120 * 1024 * 1024),
    )(A_x.reshape(S, D), A_wqkv, A_wo, B_x.reshape(S, D), B_mem0.reshape(M, D),
      B_Wq.reshape(D * HB, DB), B_Wk.reshape(D * HB, DB), B_Wv.reshape(D * HB, DB),
      B_Wo.reshape(HB * DB, D))
    return out.reshape(1, S, 2 * D)
```

```python
import functools
import math

import jax
import jax.numpy as jnp
from jax import lax
import jax.experimental.pallas as pl
import jax.experimental.pallas.tpu as pltpu

bf16 = jnp.bfloat16
f32 = jnp.float32
u32 = jnp.uint32

S = 2048
D = 1024
HA, DA = 32, 32
HB, DB = 32, 128
M, SEG = 8, 32
L = M + SEG
NSEG = S // SEG

QB = 512
QP = QB // 2
NQB = S // QB
KT = 128
NKT = S // KT
NB = HA * NQB // 4
TREE = 4

G = 4
UNROLL = 2
NAP = 2

NWC = 4
WC = D // NWC
RC = 8
NRC = D // 16 // RC
NSLOT = 3

LOG2E = math.log2(math.e)

B_ORDER = (
    ('k0 q0 q1 v0 qk0 sm0 k1 q2 qk1 pv0 sm1 v1 k2 o0b pv1 v2 qk2 o0a o1b A3 sm2 q3 pv2 k3 o1a qk3 '
     'o2a sm3 v3 q4 pv3 k4 v4 qk4 o2b o3b o3a sm4 q5 pv4 k5 o4a qk5 v5 o4b sm5 q6 pv5 k6 o5a k7 '
     'qk6 A2 sm6 v6 q7 o5b qk7 sm7 pv6 v7 o6a pv7 o6b o7a o7b A0 '),
    ('q0 k0 q1 qk0 v0 sm0 k1 q2 pv0 o0b qk1 A1 v1 sm1 k2 pv1 v2 o1b qk2 sm2 q3 o0a o1a pv2 k3 o2a '
     'qk3 v3 q4 sm3 pv3 k4 o2b o3b qk4 sm4 o3a v4 q5 pv4 k5 v5 o4a o4b qk5 k6 q6 sm5 pv5 k7 qk6 '
     'o5a sm6 v6 q7 pv6 o5b qk7 v7 sm7 o6a pv7 o6b o7b o7a '),
)
B_FIRST = (
    ('U k0 q0 q1 U v0 U qk0 sm0 U k1 q2 U qk1 U sm1 pv0 v1 k2 U pv1 A1 o0b U v2 U o0a qk2 U o1b A3 '
     'U q3 sm2 k3 U pv2 U qk3 U sm3 o2a o1a U A2 U v3 pv3 o2b k4 q4 v4 qk4 U U o3a U o3b sm4 U q5 '
     'pv4 k5 o4a U qk5 U o4b v5 sm5 U q6 pv5 k6 U U k7 qk6 U o5a sm6 v6 U q7 U U pv6 o5b qk7 U v7 '
     'sm7 o6a A0 U pv7 o6b U o7a o7b U U '),
    ('q0 U U k0 q1 qk0 U v0 U k1 q2 U sm0 pv0 o0b qk1 U sm1 U v1 U k2 pv1 U v2 o1b U qk2 sm2 q3 U '
     'o0a o1a U pv2 U k3 o2a U U qk3 v3 q4 sm3 U pv3 k4 U o2b o3b U qk4 sm4 U o3a v4 U q5 pv4 U k5 '
     'v5 U o4a o4b U qk5 k6 U q6 sm5 pv5 U k7 U qk6 U U v6 o5b q7 sm6 pv6 o5a U qk7 U sm7 v7 o6a '
     'pv7 o6b o7b o7a '),
)


def _parse_order(txt):
    out = []
    for t in txt.split():
        if t == 'U':
            out.append(('U', 0, ''))
            continue
        part = t[-1] if t[-1] in 'ab' else ''
        t = t[:-1] if part else t
        out.append((t[:-1], int(t[-1]), part))
    return out


def _pk(x):
    return pltpu.bitcast(x, u32)


def _up(x):
    return pltpu.bitcast(x, bf16)


def _dot(a, b):
    return jnp.dot(a, b, preferred_element_type=f32)


def _kernel(xa_hbm, wqkv_hbm, woa_hbm, xb_hbm, mem0_hbm, wq_hbm, wk_hbm, wv_hbm, wob_hbm,
            out_hbm,
            xa, wqkv, woa, k3, qvt, tstage, oa, s0, s1, s2, s3, s4, s5, s6, s7, m_ref, os0, os1,
            wq, wk, wv, wob, xb, raw, outa, outb, h_ref, mem0, z_ref, sems, rsems, osems):
    qt = qvt.at[0]
    vt = qvt.at[1]
    z_ref[...] = jnp.zeros(z_ref.shape, u32)

    xa32 = xa_hbm.bitcast(u32)
    wqkv32 = wqkv_hbm.bitcast(u32)

    def cp_x0(hf):
        rows = pl.ds(hf * (QP // 2), QP // 2)
        return pltpu.make_async_copy(xa32.at[rows, :], xa.at[rows, :], sems.at[(0, 13)[hf]])

    def cp_xa(r):
        rows = pl.ds(r * QP, QP)
        return pltpu.make_async_copy(xa32.at[rows, :], xa.at[rows, :], sems.at[r])

    def cp_wq(c):
        cols = pl.ds(c * WC, WC)
        return pltpu.make_async_copy(wqkv32.at[:, cols], wqkv.at[:, cols], sems.at[4 + c])

    def cp_wkv(i):
        cols = pl.ds(i * D, D)
        return pltpu.make_async_copy(wqkv32.at[:, cols], wqkv.at[:, cols], sems.at[7 + i])

    cp_woa = pltpu.make_async_copy(woa_hbm.bitcast(u32), woa, sems.at[10])
    cp_xb = pltpu.make_async_copy(xb_hbm.bitcast(u32), xb, sems.at[11])
    cp_wob = pltpu.make_async_copy(wob_hbm.bitcast(u32), wob, sems.at[12])
    cp_mem0 = pltpu.make_async_copy(mem0_hbm, mem0, sems.at[14])

    w_hbms = (wq_hbm, wk_hbm, wv_hbm)
    w_dsts = (wq, wk, wv)

    def raw_copy(c, i):
        return pltpu.make_async_copy(
            w_hbms[i].bitcast(u32).at[pl.ds(c * (RC * 256), RC * 256), :],
            raw.at[c % NSLOT, i], rsems.at[c % NSLOT, i])

    def raw_start(c):
        for i in range(3):
            raw_copy(c, i).start()

    def raw_step(c):
        for i in range(3):
            raw_copy(c, i).wait()

        @pl.when(c + NSLOT - 1 < NRC)
        def _():
            raw_start(c + NSLOT - 1)

    def relayout_chunk(c):
        slot = c % NSLOT
        z = z_ref[...]
        hm = jnp.uint32(0xFFFF0000)
        prev = None
        for t in range(RC):
            rows = pl.ds(pl.multiple_of((c * RC + t) * 8, 8), 8)
            for i in range(3):
                for j in range(HB // 2):
                    a = raw[slot, i, pl.ds(t * 256 + j, 8, stride=16), :]
                    b = raw[slot, i, pl.ds(t * 256 + 128 + j, 8, stride=16), :]
                    if prev is not None:
                        pz = prev & z
                        a = a | pz
                        b = b | pz
                    lo = jnp.concatenate([pltpu.bitcast(a << 16, f32), pltpu.bitcast(b << 16, f32)], axis=0)
                    hi = jnp.concatenate([pltpu.bitcast(a & hm, f32), pltpu.bitcast(b & hm, f32)], axis=0)
                    lo = _pk(lo.astype(bf16))
                    hi = _pk(hi.astype(bf16))
                    w_dsts[i][rows, (2 * j) * DB:(2 * j + 1) * DB] = lo
                    w_dsts[i][rows, (2 * j + 1) * DB:(2 * j + 2) * DB] = hi
                    prev = hi

    qscale = DA ** -0.5 * LOG2E

    def xrows(r):
        return _up(xa[pl.ds(pl.multiple_of(r * QP, QP), QP), :])

    def q_dot(x_, c0, nc):
        return _dot(x_, _up(wqkv[:, c0:c0 + nc])) * qscale

    def t_stage(y, r0, c0):
        tstage[r0 // 2:(r0 + y.shape[0]) // 2, c0:c0 + y.shape[1]] = _pk(y.astype(bf16))

    def t_flush(which, r):
        for g in range(8):
            t = _up(tstage[:, g * 128:(g + 1) * 128]).astype(f32).T.astype(bf16)
            qvt[which, r, g * 4:g * 4 + 4] = _pk(t).reshape(4, DA // 2, QB)

    def a1_q(r, c):
        cp_xa(r).wait()
        t_flush(0, r - 1)
        t_stage(q_dot(xrows(r), 0, D), 0, 0)
        return c

    def a1_k(r, c):
        raw_step(r)
        k = _dot(xrows(r), _up(wqkv[:, D:2 * D])).astype(bf16)
        for g in range(8):
            k3[g, pl.ds(pl.multiple_of(r * QP, QP), QP), :] = _pk(k[:, g * 128:(g + 1) * 128])
        relayout_chunk(r)
        return c

    def a1_v(r, c):
        raw_step(NQB + r)
        t_flush(jnp.where(r == 0, 0, 1), jnp.where(r == 0, NQB - 1, r - 1))
        t_stage(_dot(xrows(r), _up(wqkv[:, 2 * D:3 * D])), 0, 0)
        relayout_chunk(NQB + r)
        return c

    cp_wq(0).start()
    cp_x0(0).start()
    cp_x0(1).start()
    for c in range(1, NWC):
        cp_wq(c).start()
    for r in range(1, NQB):
        cp_xa(r).start()
    cp_wkv(1).start()
    raw_start(0)
    cp_wkv(2).start()
    for c in range(1, NSLOT - 1):
        raw_start(c)

    def x0half(hf):
        return _up(xa[hf * (QP // 2):(hf + 1) * (QP // 2), :])

    pieces = [(cp_x0(0), lambda: x0half(0), 0, 0), (cp_x0(1), lambda: x0half(1), QB // 2, 0)]
    pieces += [(cp_wq(c), lambda: xrows(0), 0, c * WC) for c in range(1, NWC)]
    cp_wq(0).wait()
    prev = None
    for cp, lhs, r0, c0 in pieces:
        cp.wait()
        y = q_dot(lhs(), c0, WC)
        if prev is not None:
            t_stage(*prev)
        prev = (y, r0, c0)
    t_stage(*prev)

    lax.fori_loop(1, NQB, a1_q, 0)
    cp_wkv(1).wait()
    lax.fori_loop(0, NQB, a1_k, 0)
    cp_wkv(2).wait()
    lax.fori_loop(0, NQB, a1_v, 0)
    cp_woa.start()
    cp_xb.start()
    cp_wob.start()
    cp_mem0.start()

    sbufs = (s0, s1, s2, s3, s4, s5, s6, s7)

    def probs(sr, kt, m2):
        p = jnp.exp2(sr[kt * KT:(kt + 1) * KT, :] - m2)
        t = p.reshape(KT // 8, 8, QB)
        for _ in range(TREE):
            t4 = t.reshape(t.shape[0] // 2, 2, 8, QB)
            t = t4[:, 0] + t4[:, 1]
        return p.astype(bf16), jnp.sum(t, axis=0)

    def vt_tile(h, kt):
        r_, c_ = divmod(kt * KT, QB)
        return _up(vt[r_, h, :, c_:c_ + KT])

    def item(hh, b1, sw, b2, sr, m2, ostage, produce, consume):
        m = acc = l = None
        if produce:
            g1 = b1 // NQB
            parts = []
            if hh > 0:
                parts.append(jnp.zeros((DA * hh, QB), bf16))
            parts.append(_up(qt[b1 % NQB, g1 * 4 + hh]))
            if hh < 3:
                parts.append(jnp.zeros((DA * (3 - hh), QB), bf16))
            q_ = jnp.concatenate(parts, axis=0)
        if consume:
            h2 = (b2 // NQB) * 4 + hh
        for kt in range(NKT):
            if produce:
                st = _dot(_up(k3[g1, kt * (KT // 2):(kt + 1) * (KT // 2), :]), q_)
                sw[kt * KT:(kt + 1) * KT, :] = st
                mm = jnp.max(st.reshape(KT // 8, 8, QB), axis=0)
                m = mm if m is None else jnp.maximum(m, mm)
            if consume:
                p, ll = probs(sr, kt, m2)
                l = ll if l is None else l + ll
                o = _dot(vt_tile(h2, kt), p)
                acc = o if acc is None else acc + o
        if consume:
            ostage[hh * DA:(hh + 1) * DA, :] = acc * (1.0 / jnp.sum(l, axis=0, keepdims=True))
        if produce:
            return jnp.max(m, axis=0, keepdims=True)

    def flush_o(b, ostage):
        b = jnp.maximum(b, 0)
        oa[b // NQB, pl.ds(pl.multiple_of((b % NQB) * QP, QP), QP), :] = _pk(ostage[...].T.astype(bf16))

    def block(b, par, consume=True):
        if consume:
            flush_o(b - 1, (os0, os1)[1 - par])
        b1 = jnp.minimum(b + 1, NB - 1)
        for j in range(4):
            m2 = m_ref[par * 4 + j] if consume else None
            m_ref[(1 - par) * 4 + j] = item(j, b1, sbufs[(1 - par) * 4 + j], b, sbufs[par * 4 + j], m2,
                                            (os0, os1)[par], True, consume)

    def a2_body(i, c):
        block(2 * i, 0)

        @pl.when(2 * i + 1 < NB - 1)
        def _():
            block(2 * i + 1, 1)
        return c

    def last_block_units():
        b = NB - 1
        flush_o(b - 1, os0)
        for hh in range(4):
            sr = sbufs[4 + hh]
            m2 = m_ref[4 + hh]
            h2 = (b // NQB) * 4 + hh
            acc = l = None
            for kt in range(NKT):
                p, ll = probs(sr, kt, m2)
                l = ll if l is None else l + ll
                o = _dot(vt_tile(h2, kt), p)
                acc = o if acc is None else acc + o
                if kt == NKT - 1:
                    os1[hh * DA:(hh + 1) * DA, :] = acc * (1.0 / jnp.sum(l, axis=0, keepdims=True))
                yield
        flush_o(b, os1)

    t_flush(1, NQB - 1)
    block(-1, 1, consume=False)
    os1[...] = jnp.zeros(os1.shape, f32)
    lax.fori_loop(0, NB // 2, a2_body, 0)

    cp_woa.wait()
    cp_xb.wait()
    cp_wob.wait()
    cp_mem0.wait()
    scale = DB ** -0.5 * LOG2E
    h_ref[0:M, :] = mem0[...].astype(f32)
    row = lax.broadcasted_iota(jnp.int32, (L, L), 0)
    col = lax.broadcasted_iota(jnp.int32, (L, L), 1)
    mask = (row < M) | (row >= col)

    def w(ref, r0, nr, c0, nc):
        return _up(ref[r0 // 2:(r0 + nr) // 2, c0:c0 + nc])

    def a4_part(s, p):
        prow = pl.ds(pl.multiple_of(s * (SEG // 2), SEG // 2), SEG // 2)
        o_ = jnp.concatenate([_up(oa[g, prow, :]) for g in range(8)], axis=1)
        wd = D // NAP
        y = _dot(o_, _up(woa[:, p * wd:(p + 1) * wd]))
        outa[pl.ds(pl.multiple_of(s * SEG, SEG), SEG), p * wd:(p + 1) * wd] = y.astype(bf16)

    def segment(s, order, s0, side=None):
        h_ref[M:L, :] = _up(xb[pl.ds(pl.multiple_of(s * (SEG // 2), SEG // 2), SEG // 2), :]).astype(f32)
        hv = h_ref[...]
        st = {}
        acc = {}
        for op, g, part in order:
            if op == 'U':
                next(side)
            elif op == 'A':
                a4_part(s0 + g // NAP, g % NAP)
            elif op in ('q', 'k', 'v'):
                ref = {'q': wq, 'k': wk, 'v': wv}[op]
                st[op, g] = _dot(hv, w(ref, 0, D, g * G * DB, G * DB))
            elif op == 'qk':
                q = st.pop(('q', g))
                k = st.pop(('k', g))
                st['s', g] = [
                    lax.dot_general(q[:, j * DB:(j + 1) * DB], k[:, j * DB:(j + 1) * DB].astype(bf16),
                                    (((1,), (1,)), ((), ())), preferred_element_type=f32)
                    for j in range(G)]
            elif op == 'sm':
                ps = []
                for sc in st.pop(('s', g)):
                    sc = jnp.where(mask, sc * scale, -1e9)
                    p = jnp.exp2(sc - jnp.max(sc, axis=-1, keepdims=True))
                    ps.append(p / jnp.sum(p, axis=-1, keepdims=True))
                st['p', g] = ps
            elif op == 'pv':
                v = st.pop(('v', g))
                st['ov', g] = jnp.concatenate(
                    [_dot(p, v[:, j * DB:(j + 1) * DB].astype(bf16))
                     for j, p in enumerate(st.pop(('p', g)))], axis=1)
            elif op == 'o':
                hf = 'ab'.index(part)
                r = _dot(st['ov', g], w(wob, g * G * DB, G * DB, hf * (D // 2), D // 2))
                acc[hf] = r if hf not in acc else acc[hf] + r
        for hf in (0, 1):
            cols = slice(hf * (D // 2), (hf + 1) * (D // 2))
            h_ref[0:M, cols] = acc[hf][0:M, :].astype(bf16).astype(f32)
            outb[pl.ds(pl.multiple_of(s * SEG, SEG), SEG), cols] = acc[hf][M:L, :].astype(bf16)

    def out_start(i):
        rows = pl.ds(i * (UNROLL * SEG), UNROLL * SEG)
        pltpu.make_async_copy(outa.at[rows, :], out_hbm.at[rows, pl.ds(0, D)], osems.at[0]).start()
        pltpu.make_async_copy(outb.at[rows, :], out_hbm.at[rows, pl.ds(D, D)], osems.at[1]).start()

    side = last_block_units()
    for u in range(UNROLL):
        segment(u, _parse_order(B_FIRST[u]), 0, side)
    for _ in side:
        pass

    orders = [_parse_order(t) for t in B_ORDER]

    def b_body(i, c):
        out_start(i - 1)
        for u in range(UNROLL):
            segment(i * UNROLL + u, orders[u], i * UNROLL)
        return c

    lax.fori_loop(1, NSEG // UNROLL, b_body, 0)
    out_start(NSEG // UNROLL - 1)

    pltpu.make_async_copy(outa, out_hbm.at[:, pl.ds(0, D)], osems.at[0]).wait()
    pltpu.make_async_copy(outb, out_hbm.at[:, pl.ds(D, D)], osems.at[1]).wait()


@functools.partial(jax.jit, static_argnames=("B_seg_len",))
def pallas_concat_heads__softmax_full_mha__memory_aug_recurrent_mem_tr__prompt_kernel(
        A_x, A_wqkv, A_wo, B_x, B_mem0, B_Wq, B_Wk, B_Wv, B_Wo, B_seg_len):
    assert B_seg_len == SEG and A_x.shape == (1, S, D) and B_x.shape == (1, S, D)
    assert B_mem0.shape == (1, M, D) and B_Wq.shape == (D, HB, DB) and B_Wo.shape == (HB, DB, D)
    hbm = pl.BlockSpec(memory_space=pl.ANY)
    V = pltpu.VMEM
    scratch = [
        V((S // 2, D), u32),
        V((D // 2, 3 * D), u32),
        V((D // 2, D), u32),
        V((8, S // 2, 128), u32),
        V((2, NQB, HA, DA // 2, QB), u32),
        V((QB // 2, D), u32),
        V((8, S // 2, 128), u32),
    ] + [V((S, QB), f32) for _ in range(8)] + [
        V((8, 1, QB), f32),
        V((128, QB), f32), V((128, QB), f32),
        V((D // 2, HB * DB), u32),
        V((D // 2, HB * DB), u32),
        V((D // 2, HB * DB), u32),
        V((HB * DB // 2, D), u32),
        V((S // 2, D), u32),
        V((NSLOT, 3, RC * 256, 128), u32),
        V((S, D), bf16),
        V((S, D), bf16),
        V((L, D), f32),
        V((M, D), bf16),
        V((8, 128), u32),
        pltpu.SemaphoreType.DMA((15,)),
        pltpu.SemaphoreType.DMA((NSLOT, 3)),
        pltpu.SemaphoreType.DMA((2,)),
    ]
    out = pl.pallas_call(
        _kernel,
        out_shape=jax.ShapeDtypeStruct((S, 2 * D), bf16),
        in_specs=[hbm] * 9,
        out_specs=hbm,
        scratch_shapes=scratch,
        compiler_params=pltpu.CompilerParams(vmem_limit_bytes=120 * 1024 * 1024),
    )(A_x.reshape(S, D), A_wqkv, A_wo, B_x.reshape(S, D), B_mem0.reshape(M, D),
      B_Wq.reshape(D * HB, DB), B_Wk.reshape(D * HB, DB), B_Wv.reshape(D * HB, DB),
      B_Wo.reshape(HB * DB, D))
    return out.reshape(1, S, 2 * D)
```
